```python
import jax
import jax.numpy as jnp

def _softmax(x, axis=-1):
    return jax.nn.softmax(x, axis=axis)

def _gelu(x):
    return jax.nn.gelu(x, approximate=True)

def _silu(x):
    return jax.nn.silu(x)

def _sigmoid(x):
    return jax.nn.sigmoid(x)

def _layernorm(x, axis=-1, eps=1e-05):
    m = jnp.mean(x, axis=axis, keepdims=True)
    v = jnp.var(x, axis=axis, keepdims=True)
    return (x - m) / jnp.sqrt(v + eps)

def _scatter_add(tgt, idx, src, axis=0):
    return tgt.at[idx].add(src)

def _segment_sum(src, seg, n):
    return jax.ops.segment_sum(src, seg, n)

class _Rng:

    def __init__(self, key):
        self._k = key

    def _next(self):
        self._k, sub = jax.random.split(self._k)
        return sub

    def normal(self, shape):
        return jax.random.normal(self._next(), shape, dtype=jnp.bfloat16)

    def randint(self, lo, hi, shape):
        return jax.random.randint(self._next(), shape, lo, hi, dtype=jnp.int32)

    def uniform(self, shape, lo=0.0, hi=1.0):
        return jax.random.uniform(self._next(), shape, jnp.bfloat16, lo, hi)

    def permutation(self, n):
        return jax.random.permutation(self._next(), n)
kernel_name = 'concat_heads__ssm_conv_h3__memory_aug_recurrent_mem_tr__prompt'

def setup_inputs():
    _rng = _Rng(jax.random.key(int.from_bytes(__import__("os").urandom(4), "little")))
    _w = lambda a: (lambda t: t.astype(jnp.bfloat16) if jnp.issubdtype(t.dtype, jnp.floating) else t)(jnp.asarray(a))

    def _A_setup():
        B, S, D = (1, 2048, 1024)
        ks = 4
        return {'q': _w((lambda *s: _rng.normal(s) * 0.05)(B, S, D)), 'k': _w((lambda *s: _rng.normal(s) * 0.05)(B, S, D)), 'v': _w((lambda *s: _rng.normal(s) * 0.05)(B, S, D)), 'shift_k': _w((lambda *s: _rng.normal(s) * 0.05)(D, ks) * 0.5), 'ssm_k': _w((lambda *s: _rng.normal(s) * 0.05)(D, S) * (1.0 / S ** 0.5)), 'ssm_D': _w((lambda *s: _rng.normal(s) * 0.05)(D))}
    _A_in = _A_setup()

    def _B_setup():
        B, S, Dm = (1, 2048, 1024)
        H, Dh = (32, 128)
        M, seg = (8, 32)
        seg = min(seg, S)
        S = S // seg * seg
        return {'x': _w((lambda *s: _rng.normal(s) * 0.05)(B, S, Dm)), 'mem0': _w((lambda *s: _rng.normal(s) * 0.05)(B, M, Dm)), 'Wq': _w((lambda *s: _rng.normal(s) * 0.05)(Dm, H, Dh) * Dm ** (-0.5)), 'Wk': _w((lambda *s: _rng.normal(s) * 0.05)(Dm, H, Dh) * Dm ** (-0.5)), 'Wv': _w((lambda *s: _rng.normal(s) * 0.05)(Dm, H, Dh) * Dm ** (-0.5)), 'Wo': _w((lambda *s: _rng.normal(s) * 0.05)(H, Dh, Dm) * (H * Dh) ** (-0.5)), 'seg_len': seg}
    _B_in = _B_setup()
    return {'A_q': _A_in['q'], 'A_k': _A_in['k'], 'A_v': _A_in['v'], 'A_shift_k': _A_in['shift_k'], 'A_ssm_k': _A_in['ssm_k'], 'A_ssm_D': _A_in['ssm_D'], 'B_x': _B_in['x'], 'B_mem0': _B_in['mem0'], 'B_Wq': _B_in['Wq'], 'B_Wk': _B_in['Wk'], 'B_Wv': _B_in['Wv'], 'B_Wo': _B_in['Wo'], 'B_seg_len': _B_in['seg_len']}

def reference(A_q, A_k, A_v, A_shift_k, A_ssm_k, A_ssm_D, B_x, B_mem0, B_Wq, B_Wk, B_Wv, B_Wo, B_seg_len):

    def _A_ref(q, k, v, shift_k, ssm_k, ssm_D):
        B, S, D = q.shape
        ks = shift_k.shape[-1]
        k_pad = jnp.pad(k, ((0, 0), (ks - 1, 0), (0, 0)))
        k_shift = jnp.zeros_like(k)
        for t in range(ks):
            k_shift = k_shift + k_pad[:, t:t + S, :] * shift_k[:, ks - 1 - t][None, None, :]
        kv = k_shift * v
        L = 2 * S
        kv_pad = jnp.pad(kv, ((0, 0), (0, S), (0, 0)))
        kf_pad = jnp.pad(ssm_k, ((0, 0), (0, S)))
        kv_f = (lambda x, axes=(-2, -1): jnp.fft.rfft2(x.astype(jnp.float32), axes=axes))(kv_pad[:, None, :, :], axes=(1, 2))
        kf_f = (lambda x, axes=(-2, -1): jnp.fft.rfft2(x.astype(jnp.float32), axes=axes))(kf_pad[:, None, :], axes=(1, 2))
        kf_f = (lambda x, *d: x.transpose(*d))(kf_f, 1, 2, 0)
        y_f = kv_f * kf_f[None, :, :, :]
        y = (lambda x, s, axes=(-2, -1): jnp.fft.irfft2(x, s=s, axes=axes).astype(jnp.bfloat16))(y_f, (1, L), axes=(1, 2))[:, 0, :S, :]
        y = y + kv * ssm_D[None, None, :]
        return q * y

    def _B_ref(x, mem0, Wq, Wk, Wv, Wo, seg_len):
        B, S, Dm = x.shape
        H, Dh = (Wq.shape[1], Wq.shape[2])
        M = mem0.shape[1]
        scale = Dh ** (-0.5)
        n_seg = S // seg_len
        L = M + seg_len
        idx = jnp.arange(L)
        mask = (idx[:, None] < M) | (idx[:, None] >= idx[None, :])
        mem = mem0
        outs = []
        for s in range(n_seg):
            xs = x[:, s * seg_len:(s + 1) * seg_len, :].copy()
            h = jnp.concatenate([mem, xs], axis=1)
            q = jnp.einsum('btd,dhe->bhte', h, Wq)
            k = jnp.einsum('btd,dhe->bhte', h, Wk)
            v = jnp.einsum('btd,dhe->bhte', h, Wv)
            scores = jnp.einsum('bhqe,bhke->bhqk', q, k) * scale
            scores = jnp.where(mask[None, None], scores, -1000000000.0)
            p = _softmax(scores, axis=-1)
            o = jnp.einsum('bhqk,bhke->bhqe', p, v)
            o = jnp.einsum('bhte,hed->btd', o, Wo)
            mem = o[:, :M, :].copy()
            outs.append(o[:, M:, :])
        return jnp.concatenate(outs, axis=1)
    a = _A_ref(A_q, A_k, A_v, A_shift_k, A_ssm_k, A_ssm_D)
    b = _B_ref(B_x, B_mem0, B_Wq, B_Wk, B_Wv, B_Wo, B_seg_len)
    return jnp.concatenate([a, b], axis=-1)
```

```python
import functools

import jax
import jax.numpy as jnp
import numpy as np
from jax import lax
from jax.experimental import pallas as pl
from jax.experimental.pallas import tpu as pltpu

F32 = jnp.float32
BF16 = jnp.bfloat16
LANES = 128
P = 128


def _dft_matrices():
    theta = np.pi * (4 * np.arange(P) + 1) / (2 * P)
    ang = theta[:, None] * np.arange(P)[None, :]
    fwd = np.concatenate([np.cos(ang), -np.sin(ang)], axis=0)
    return fwd.astype(np.float32), (fwd.T / P).astype(np.float32)


def _nn(a, b):
    return lax.dot_general(a, b, (((1,), (0,)), ((), ())), preferred_element_type=F32)


def _nt(a, b):
    return lax.dot_general(a, b, (((1,), (1,)), ((), ())), preferred_element_type=F32)


def _kernel(
    aq_hbm, ak_hbm, av_hbm, shift_ref, ssmk_hbm, ssmd_ref, x_hbm, mem0_ref,
    wq_hbm, wk_hbm, wv_hbm, wo_hbm, fwd_ref, inv_ref,
    out_hbm,
    aq, ak, av, ssmk, aout, par, kf, kvf, ubuf, kbuf, zbuf,
    raw, wqkv, wo, xs, hbuf, obuf, bout,
    sem_a, sem_w, sem_wo, sem_x, sem_ao, sem_bo,
    *, S, D, H, M, seg,
):
    NB = D // LANES
    Q = S // P
    L = M + seg
    n_seg = S // seg
    KS = shift_ref.shape[0]
    WCH = D // NB
    w_hbm = (wq_hbm, wk_hbm, wv_hbm)

    def a_copies(c):
        cols = pl.ds(pl.multiple_of(c * LANES, LANES), LANES)
        return (
            pltpu.make_async_copy(ak_hbm.at[:, cols], ak.at[c], sem_a.at[c, 0]),
            pltpu.make_async_copy(av_hbm.at[:, cols], av.at[c], sem_a.at[c, 1]),
            pltpu.make_async_copy(ssmk_hbm.at[cols, :], ssmk.at[c], sem_a.at[c, 2]),
            pltpu.make_async_copy(aq_hbm.at[:, cols], aq.at[c], sem_a.at[c, 3]),
        )

    def w_copies(c):
        rows = pl.ds(pl.multiple_of(c * WCH * H, WCH * H), WCH * H)
        return tuple(
            pltpu.make_async_copy(w_hbm[m].at[rows, :], raw.at[m, rows, :], sem_w.at[c, m])
            for m in range(3)
        )

    def wo_copy(c):
        cols = pl.ds(pl.multiple_of(c * LANES, LANES), LANES)
        return pltpu.make_async_copy(wo_hbm.at[:, cols], wo.at[c], sem_wo.at[c])

    def aout_copy(c):
        cols = pl.ds(pl.multiple_of(c * LANES, LANES), LANES)
        return pltpu.make_async_copy(aout.at[c], out_hbm.at[:, cols], sem_ao.at[c])

    XG = 8
    XR = S // XG

    def x_copy(g):
        rows = pl.ds(pl.multiple_of(g * XR, XR), XR)
        return pltpu.make_async_copy(x_hbm.at[rows, :], xs.at[rows, :], sem_x.at[g])

    def bout_copy(g):
        rows = pl.ds(pl.multiple_of(g * XR, XR), XR)
        return pltpu.make_async_copy(
            bout.at[rows, :], out_hbm.at[rows, pl.ds(D, D)], sem_bo.at[g])

    def head_a(c, w, dskip):
        ck, cv, cs, cq = a_copies(c)
        ck.wait()
        kf[pl.ds(8, S), :] = ak[c].astype(F32)
        cv.wait()
        fwd = fwd_ref[...]
        for i in range(Q):
            acc = kf[pl.ds(8 + i * P - (KS - 1), P), :] * w[KS - 1]
            for j in range(KS - 2, -1, -1):
                acc = acc + kf[pl.ds(8 + i * P - j, P), :] * w[j]
            kv = (acc * av[c, pl.ds(i * P, P), :].astype(F32)).astype(BF16)
            kvf[pl.ds(i * P, P), :] = kv
            ubuf[i] = _nn(fwd, kv)
        cs.wait()
        for j in range(Q):
            kbuf[j] = _nt(fwd, ssmk[c, :, pl.ds(j * P, P)])

        def conv(p, _):
            re = pl.ds(pl.multiple_of(p * 8, 8), 8)
            im = pl.ds(pl.multiple_of(P + p * 8, 8), 8)
            ua = [ubuf[i, re, :] for i in range(Q)]
            ub = [ubuf[i, im, :] for i in range(Q)]
            kc = [kbuf[0, re, :]] + [kbuf[j, re, :] - kbuf[j - 1, im, :] for j in range(1, Q)]
            kd = [kbuf[0, im, :]] + [kbuf[j, im, :] + kbuf[j - 1, re, :] for j in range(1, Q)]
            us = [a + b for a, b in zip(ua, ub)]
            s1 = []
            for a in range(Q):
                t = kc[0] * us[a]
                for j in range(1, a + 1):
                    t = t + kc[j] * us[a - j]
                s1.append(t)
            km = [d_ - c_ for c_, d_ in zip(kc, kd)]
            for a in range(Q):
                t = s1[a]
                for j in range(a + 1):
                    t = t + km[j] * ua[a - j]
                zbuf[a, im, :] = t
            kp = [d_ + c_ for c_, d_ in zip(kc, kd)]
            for a in range(Q):
                t = s1[a]
                for j in range(a + 1):
                    t = t - kp[j] * ub[a - j]
                zbuf[a, re, :] = t
            return 0

        lax.fori_loop(0, P // 8, conv, 0)
        cq.wait()
        inv = inv_ref[...]
        for a in range(Q):
            rows = pl.ds(a * P, P)
            y = _nn(inv, zbuf[a].astype(BF16)) + kvf[rows, :].astype(F32) * dskip
            aout[c, rows, :] = (aq[c, rows, :].astype(F32) * y).astype(BF16)

    raw32 = raw.bitcast(jnp.uint32)

    def relayout(c):
        for cp in w_copies(c):
            cp.wait()

        def body(t, _):
            d0 = pl.multiple_of(c * WCH + t * 16, 16)
            r0 = pl.multiple_of(d0 * (H // 2), 8 * H)
            for m in range(3):
                blk = raw32[m, pl.ds(r0, 8 * H), :].reshape(16, H // 2, LANES)
                blk = jnp.swapaxes(blk, 0, 1)
                for hp in range(H // 2):
                    pair = blk[hp]
                    lo = pltpu.bitcast(pair << 16, F32).astype(BF16)
                    hi = pltpu.bitcast(pair & np.uint32(0xFFFF0000), F32).astype(BF16)
                    wqkv[m * H + 2 * hp, pl.ds(d0, 16), :] = lo
                    wqkv[m * H + 2 * hp + 1, pl.ds(d0, 16), :] = hi
            return 0

        lax.fori_loop(0, WCH // 16, body, 0)

    for cp in a_copies(0):
        cp.start()
    for cp in w_copies(0):
        cp.start()
    for cp in a_copies(1):
        cp.start()
    kf[pl.ds(0, 8), :] = jnp.zeros((8, LANES), F32)
    shift = shift_ref[...].astype(F32)
    dall = ssmd_ref[...].astype(F32)
    for c in range(NB):
        for j in range(KS):
            par[c, j] = jnp.broadcast_to(shift[j:j + 1, c * LANES:(c + 1) * LANES], (8, LANES))
        par[c, KS] = jnp.broadcast_to(dall[c:c + 1, :], (8, LANES))

    def prologue(c, _):
        @pl.when(c + 1 < NB)
        def _():
            for cp in w_copies(c + 1):
                cp.start()

        @pl.when(c + 2 < NB)
        def _():
            for cp in a_copies(c + 2):
                cp.start()

        wo_copy(c).start()

        @pl.when(c == NB - 1)
        def _():
            x_copy(0).start()

        w = [jnp.tile(par[c, j], (P // 8, 1)) for j in range(KS + 1)]
        head_a(c, w[:KS], w[KS])
        relayout(c)
        return 0

    lax.fori_loop(0, NB, prologue, 0)
    for c in range(NB):
        wo_copy(c).wait()
    for g in range(1, XG):
        x_copy(g).start()
    for c in range(NB):
        aout_copy(c).start()

    scale = LANES ** -0.5
    row = lax.broadcasted_iota(jnp.int32, (L, L), 0)
    col = lax.broadcasted_iota(jnp.int32, (L, L), 1)
    mask = (row < M) | (row >= col)
    hbuf[pl.ds(0, M), :] = mem0_ref[...].astype(F32)
    SPG = XR // seg

    def segment(s, _):
        @pl.when(s % SPG == 0)
        def _():
            x_copy(s // SPG).wait()

        rows = pl.ds(pl.multiple_of(s * seg, seg), seg)
        hbuf[pl.ds(M, seg), :] = xs[rows, :].astype(F32)
        h = hbuf[pl.ds(0, L), :]

        proj, prob = {}, {}
        for t in range(H + 2):
            if t < H:
                q = _nn(h, wqkv[t])
                k = _nn(h, wqkv[H + t]).astype(BF16)
                v = _nn(h, wqkv[2 * H + t]).astype(BF16)
                proj[t] = (q, k, v)
            if 0 <= t - 1 < H:
                q, k, v = proj.pop(t - 1)
                sc = jnp.where(mask, _nt(q, k) * scale, -1e9)
                e = jnp.exp(sc - jnp.max(sc, axis=-1, keepdims=True))
                prob[t - 1] = (e / jnp.sum(e, axis=-1, keepdims=True), v)
            if 0 <= t - 2 < H:
                p, v = prob.pop(t - 2)
                obuf[:, pl.ds((t - 2) * LANES, LANES)] = _nn(p, v)

        o = obuf[...]
        for j in range(NB):
            res = _nn(o, wo[j])
            hbuf[pl.ds(0, M), pl.ds(j * LANES, LANES)] = res[:M]
            bout[rows, pl.ds(j * LANES, LANES)] = res[M:].astype(BF16)

        @pl.when(s % SPG == SPG - 1)
        def _():
            bout_copy(s // SPG).start()

        return 0

    lax.fori_loop(0, n_seg, segment, 0)
    for c in range(NB):
        aout_copy(c).wait()
    for g in range(XG):
        bout_copy(g).wait()


@functools.partial(jax.jit, static_argnames=("B_seg_len",))
def pallas_concat_heads__ssm_conv_h3__memory_aug_recurrent_mem_tr__prompt_kernel(
    A_q, A_k, A_v, A_shift_k, A_ssm_k, A_ssm_D,
    B_x, B_mem0, B_Wq, B_Wk, B_Wv, B_Wo, B_seg_len,
):
    B, S, D = A_q.shape
    _, H, Dh = B_Wq.shape
    M = B_mem0.shape[1]
    seg = int(B_seg_len)
    assert B == 1 and Dh == LANES and B_x.shape == (B, S, D)
    NB = D // LANES
    Q = S // P
    fwd, inv = _dft_matrices()

    hbm = pl.BlockSpec(memory_space=pl.ANY)
    vmem = pl.BlockSpec(memory_space=pltpu.VMEM)
    out = pl.pallas_call(
        functools.partial(_kernel, S=S, D=D, H=H, M=M, seg=seg),
        out_shape=jax.ShapeDtypeStruct((S, 2 * D), BF16),
        in_specs=[hbm, hbm, hbm, vmem, hbm, vmem, hbm, vmem, hbm, hbm, hbm, hbm, vmem, vmem],
        out_specs=hbm,
        scratch_shapes=[
            pltpu.VMEM((NB, S, LANES), BF16),
            pltpu.VMEM((NB, S, LANES), BF16),
            pltpu.VMEM((NB, S, LANES), BF16),
            pltpu.VMEM((NB, LANES, S), BF16),
            pltpu.VMEM((NB, S, LANES), BF16),
            pltpu.VMEM((NB, A_shift_k.shape[1] + 1, 8, LANES), F32),
            pltpu.VMEM((8 + S, LANES), F32),
            pltpu.VMEM((S, LANES), BF16),
            pltpu.VMEM((Q, 2 * P, LANES), F32),
            pltpu.VMEM((Q, 2 * P, LANES), F32),
            pltpu.VMEM((Q, 2 * P, LANES), F32),
            pltpu.VMEM((3, D * H, LANES), BF16),
            pltpu.VMEM((3 * H, D, LANES), BF16),
            pltpu.VMEM((NB, H * Dh, LANES), BF16),
            pltpu.VMEM((S, D), BF16),
            pltpu.VMEM((M + seg, D), F32),
            pltpu.VMEM((M + seg, H * Dh), F32),
            pltpu.VMEM((S, D), BF16),
            pltpu.SemaphoreType.DMA((NB, 4)),
            pltpu.SemaphoreType.DMA((NB, 3)),
            pltpu.SemaphoreType.DMA((NB,)),
            pltpu.SemaphoreType.DMA((8,)),
            pltpu.SemaphoreType.DMA((NB,)),
            pltpu.SemaphoreType.DMA((8,)),
        ],
        compiler_params=pltpu.CompilerParams(vmem_limit_bytes=120 * 1024 * 1024),
        name="h3_rmt_concat",
    )(
        A_q.reshape(S, D), A_k.reshape(S, D), A_v.reshape(S, D),
        A_shift_k.T, A_ssm_k, A_ssm_D.reshape(NB, LANES),
        B_x.reshape(S, D), B_mem0.reshape(M, D),
        B_Wq.reshape(D * H, Dh), B_Wk.reshape(D * H, Dh), B_Wv.reshape(D * H, Dh),
        B_Wo.reshape(H * Dh, D),
        fwd.astype(BF16), inv.astype(BF16),
    )
    return out.reshape(B, S, 2 * D)
```

```python
import functools

import jax
import jax.numpy as jnp
import numpy as np
from jax import lax
from jax.experimental import pallas as pl
from jax.experimental.pallas import tpu as pltpu

F32 = jnp.float32
BF16 = jnp.bfloat16
LANES = 128
P = 128


def _dft_matrices():
    theta = np.pi * (4 * np.arange(P) + 1) / (2 * P)
    ang = theta[:, None] * np.arange(P)[None, :]
    fwd = np.concatenate([np.cos(ang), -np.sin(ang)], axis=0)
    return fwd.astype(np.float32), (fwd.T / P).astype(np.float32)


def _nn(a, b):
    return lax.dot_general(a, b, (((1,), (0,)), ((), ())), preferred_element_type=F32)


def _nt(a, b):
    return lax.dot_general(a, b, (((1,), (1,)), ((), ())), preferred_element_type=F32)


def _kernel(
    aq_hbm, ak_hbm, av_hbm, shift_ref, ssmk_hbm, ssmd_ref, x_hbm, mem0_ref,
    wq_hbm, wk_hbm, wv_hbm, wo_hbm, fwd_ref, inv_ref,
    out_hbm,
    aq, ak, av, ssmk, aout, par, kf, kvf, ubuf, kbuf, zbuf,
    raw, wqkv, wo, xs, hbuf, obuf, bout,
    sem_a, sem_w, sem_wo, sem_x, sem_ao, sem_bo,
    *, S, D, H, M, seg,
):
    NB = D // LANES
    Q = S // P
    L = M + seg
    n_seg = S // seg
    KS = shift_ref.shape[0]
    WCH = D // NB
    w_hbm = (wq_hbm, wk_hbm, wv_hbm)

    def a_copies(c):
        cols = pl.ds(pl.multiple_of(c * LANES, LANES), LANES)
        return (
            pltpu.make_async_copy(ak_hbm.at[:, cols], ak.at[c], sem_a.at[c, 0]),
            pltpu.make_async_copy(av_hbm.at[:, cols], av.at[c], sem_a.at[c, 1]),
            pltpu.make_async_copy(ssmk_hbm.at[cols, :], ssmk.at[c], sem_a.at[c, 2]),
            pltpu.make_async_copy(aq_hbm.at[:, cols], aq.at[c], sem_a.at[c, 3]),
        )

    def w_copies(c):
        rows = pl.ds(pl.multiple_of(c * WCH * H, WCH * H), WCH * H)
        return tuple(
            pltpu.make_async_copy(w_hbm[m].at[rows, :], raw.at[m, rows, :], sem_w.at[c, m])
            for m in range(3)
        )

    def wo_copy(c):
        cols = pl.ds(pl.multiple_of(c * LANES, LANES), LANES)
        return pltpu.make_async_copy(wo_hbm.at[:, cols], wo.at[c], sem_wo.at[c])

    def aout_copy(c):
        cols = pl.ds(pl.multiple_of(c * LANES, LANES), LANES)
        return pltpu.make_async_copy(aout.at[c], out_hbm.at[:, cols], sem_ao.at[c])

    XG = 8
    XR = S // XG

    def x_copy(g):
        rows = pl.ds(pl.multiple_of(g * XR, XR), XR)
        return pltpu.make_async_copy(x_hbm.at[rows, :], xs.at[rows, :], sem_x.at[g])

    def bout_copy(g):
        rows = pl.ds(pl.multiple_of(g * XR, XR), XR)
        return pltpu.make_async_copy(
            bout.at[rows, :], out_hbm.at[rows, pl.ds(D, D)], sem_bo.at[g])

    def head_a(c, w, dskip):
        ck, cv, cs, cq = a_copies(c)
        ck.wait()
        kf[pl.ds(8, S), :] = ak[c].astype(F32)
        cv.wait()
        fwd = fwd_ref[...]
        for i in range(Q):
            acc = kf[pl.ds(8 + i * P - (KS - 1), P), :] * w[KS - 1]
            for j in range(KS - 2, -1, -1):
                acc = acc + kf[pl.ds(8 + i * P - j, P), :] * w[j]
            kv = (acc * av[c, pl.ds(i * P, P), :].astype(F32)).astype(BF16)
            kvf[pl.ds(i * P, P), :] = kv
            ubuf[i] = _nn(fwd, kv)
        cs.wait()
        for j in range(Q):
            kbuf[j] = _nt(fwd, ssmk[c, :, pl.ds(j * P, P)])

        def conv(p, _):
            re = pl.ds(pl.multiple_of(p * 8, 8), 8)
            im = pl.ds(pl.multiple_of(P + p * 8, 8), 8)
            ua = [ubuf[i, re, :] for i in range(Q)]
            ub = [ubuf[i, im, :] for i in range(Q)]
            kc = [kbuf[0, re, :]] + [kbuf[j, re, :] - kbuf[j - 1, im, :] for j in range(1, Q)]
            kd = [kbuf[0, im, :]] + [kbuf[j, im, :] + kbuf[j - 1, re, :] for j in range(1, Q)]
            us = [a + b for a, b in zip(ua, ub)]
            s1 = []
            for a in range(Q):
                t = kc[0] * us[a]
                for j in range(1, a + 1):
                    t = t + kc[j] * us[a - j]
                s1.append(t)
            km = [d_ - c_ for c_, d_ in zip(kc, kd)]
            for a in range(Q):
                t = s1[a]
                for j in range(a + 1):
                    t = t + km[j] * ua[a - j]
                zbuf[a, im, :] = t
            kp = [d_ + c_ for c_, d_ in zip(kc, kd)]
            for a in range(Q):
                t = s1[a]
                for j in range(a + 1):
                    t = t - kp[j] * ub[a - j]
                zbuf[a, re, :] = t
            return 0

        lax.fori_loop(0, P // 8, conv, 0)
        cq.wait()
        inv = inv_ref[...]
        for a in range(Q):
            rows = pl.ds(a * P, P)
            y = _nn(inv, zbuf[a].astype(BF16)) + kvf[rows, :].astype(F32) * dskip
            aout[c, rows, :] = (aq[c, rows, :].astype(F32) * y).astype(BF16)

    raw32 = raw.bitcast(jnp.uint32)

    def relayout(c):
        for cp in w_copies(c):
            cp.wait()

        def body(t, _):
            d0 = pl.multiple_of(c * WCH + t * 16, 16)
            r0 = pl.multiple_of(d0 * (H // 2), 8 * H)
            for m in range(3):
                blk = raw32[m, pl.ds(r0, 8 * H), :].reshape(16, H // 2, LANES)
                blk = jnp.swapaxes(blk, 0, 1)
                for hp in range(H // 2):
                    pair = blk[hp]
                    lo = pltpu.bitcast(pair << 16, F32).astype(BF16)
                    hi = pltpu.bitcast(pair & np.uint32(0xFFFF0000), F32).astype(BF16)
                    wqkv[m * H + 2 * hp, pl.ds(d0, 16), :] = lo
                    wqkv[m * H + 2 * hp + 1, pl.ds(d0, 16), :] = hi
            return 0

        lax.fori_loop(0, WCH // 16, body, 0)

    for cp in a_copies(0):
        cp.start()
    for cp in w_copies(0):
        cp.start()
    for cp in a_copies(1):
        cp.start()
    kf[pl.ds(0, 8), :] = jnp.zeros((8, LANES), F32)
    shift = shift_ref[...].astype(F32)
    dall = ssmd_ref[...].astype(F32)
    for c in range(NB):
        for j in range(KS):
            par[c, j] = jnp.broadcast_to(shift[j:j + 1, c * LANES:(c + 1) * LANES], (8, LANES))
        par[c, KS] = jnp.broadcast_to(dall[c:c + 1, :], (8, LANES))

    def prologue(c, _):
        @pl.when(c + 1 < NB)
        def _():
            for cp in w_copies(c + 1):
                cp.start()

        @pl.when(c + 2 < NB)
        def _():
            for cp in a_copies(c + 2):
                cp.start()

        wo_copy(c).start()

        @pl.when(c == NB - 1)
        def _():
            x_copy(0).start()

        w = [jnp.tile(par[c, j], (P // 8, 1)) for j in range(KS + 1)]
        head_a(c, w[:KS], w[KS])
        relayout(c)
        return 0

    lax.fori_loop(0, NB, prologue, 0)
    for c in range(NB):
        wo_copy(c).wait()
    for g in range(1, XG):
        x_copy(g).start()
    for c in range(NB):
        aout_copy(c).start()

    scale = LANES ** -0.5
    row = lax.broadcasted_iota(jnp.int32, (L, L), 0)
    col = lax.broadcasted_iota(jnp.int32, (L, L), 1)
    mask = (row < M) | (row >= col)
    hbuf[pl.ds(0, M), :] = mem0_ref[...].astype(F32)
    SPG = XR // seg
    wqkv32 = wqkv.bitcast(jnp.uint32)
    wo32 = wo.bitcast(jnp.uint32)

    def segment(s, _):
        @pl.when(s % SPG == 0)
        def _():
            x_copy(s // SPG).wait()

        rows = pl.ds(pl.multiple_of(s * seg, seg), seg)
        hbuf[pl.ds(M, seg), :] = xs[rows, :].astype(F32)
        h = hbuf[pl.ds(0, L), :]

        D1, D2 = 2, 4
        HS = H - 8
        proj, prob, acc, heads = {}, {}, {}, []
        for t in range(H + D2):
            if t < H:
                q = _nn(h, pltpu.bitcast(wqkv32[t], BF16))
                k = _nn(h, pltpu.bitcast(wqkv32[H + t], BF16)).astype(BF16)
                v = _nn(h, pltpu.bitcast(wqkv32[2 * H + t], BF16)).astype(BF16)
                proj[t] = (q, k, v)
            else:
                for j in range((t - H) * NB // D2, (t - H + 1) * NB // D2):
                    acc[j] = _nn(jnp.concatenate(heads[:HS], axis=1),
                                 pltpu.bitcast(wo32[j, :HS * LANES // 2, :], BF16))
            if 0 <= t - D1 < H:
                q, k, v = proj.pop(t - D1)
                sc = jnp.where(mask, _nt(q, k) * scale, -1e9)
                e = jnp.exp(sc - jnp.max(sc, axis=-1, keepdims=True))
                prob[t - D1] = (e / jnp.sum(e, axis=-1, keepdims=True), v)
            due = [u for u in prob if u <= (t - D2 if t < H + D2 - 2 else H)]
            for u in due:
                p, v = prob.pop(u)
                heads.append(_nn(p, v))

        for j in range(NB):
            res = _nn(jnp.concatenate(heads[HS:], axis=1),
                      pltpu.bitcast(wo32[j, HS * LANES // 2:, :], BF16)) + acc[j]
            hbuf[pl.ds(0, M), pl.ds(j * LANES, LANES)] = res[:M]
            bout[rows, pl.ds(j * LANES, LANES)] = res[M:].astype(BF16)

        @pl.when(s % SPG == SPG - 1)
        def _():
            bout_copy(s // SPG).start()

        return 0

    lax.fori_loop(0, n_seg, segment, 0)
    for c in range(NB):
        aout_copy(c).wait()
    for g in range(XG):
        bout_copy(g).wait()


@functools.partial(jax.jit, static_argnames=("B_seg_len",))
def pallas_concat_heads__ssm_conv_h3__memory_aug_recurrent_mem_tr__prompt_kernel(
    A_q, A_k, A_v, A_shift_k, A_ssm_k, A_ssm_D,
    B_x, B_mem0, B_Wq, B_Wk, B_Wv, B_Wo, B_seg_len,
):
    B, S, D = A_q.shape
    _, H, Dh = B_Wq.shape
    M = B_mem0.shape[1]
    seg = int(B_seg_len)
    assert B == 1 and Dh == LANES and B_x.shape == (B, S, D)
    NB = D // LANES
    Q = S // P
    fwd, inv = _dft_matrices()

    hbm = pl.BlockSpec(memory_space=pl.ANY)
    vmem = pl.BlockSpec(memory_space=pltpu.VMEM)
    out = pl.pallas_call(
        functools.partial(_kernel, S=S, D=D, H=H, M=M, seg=seg),
        out_shape=jax.ShapeDtypeStruct((S, 2 * D), BF16),
        in_specs=[hbm, hbm, hbm, vmem, hbm, vmem, hbm, vmem, hbm, hbm, hbm, hbm, vmem, vmem],
        out_specs=hbm,
        scratch_shapes=[
            pltpu.VMEM((NB, S, LANES), BF16),
            pltpu.VMEM((NB, S, LANES), BF16),
            pltpu.VMEM((NB, S, LANES), BF16),
            pltpu.VMEM((NB, LANES, S), BF16),
            pltpu.VMEM((NB, S, LANES), BF16),
            pltpu.VMEM((NB, A_shift_k.shape[1] + 1, 8, LANES), F32),
            pltpu.VMEM((8 + S, LANES), F32),
            pltpu.VMEM((S, LANES), BF16),
            pltpu.VMEM((Q, 2 * P, LANES), F32),
            pltpu.VMEM((Q, 2 * P, LANES), F32),
            pltpu.VMEM((Q, 2 * P, LANES), F32),
            pltpu.VMEM((3, D * H, LANES), BF16),
            pltpu.VMEM((3 * H, D, LANES), BF16),
            pltpu.VMEM((NB, H * Dh, LANES), BF16),
            pltpu.VMEM((S, D), BF16),
            pltpu.VMEM((M + seg, D), F32),
            pltpu.VMEM((M + seg, H * Dh), F32),
            pltpu.VMEM((S, D), BF16),
            pltpu.SemaphoreType.DMA((NB, 4)),
            pltpu.SemaphoreType.DMA((NB, 3)),
            pltpu.SemaphoreType.DMA((NB,)),
            pltpu.SemaphoreType.DMA((8,)),
            pltpu.SemaphoreType.DMA((NB,)),
            pltpu.SemaphoreType.DMA((8,)),
        ],
        compiler_params=pltpu.CompilerParams(vmem_limit_bytes=120 * 1024 * 1024),
        name="h3_rmt_concat",
    )(
        A_q.reshape(S, D), A_k.reshape(S, D), A_v.reshape(S, D),
        A_shift_k.T, A_ssm_k, A_ssm_D.reshape(NB, LANES),
        B_x.reshape(S, D), B_mem0.reshape(M, D),
        B_Wq.reshape(D * H, Dh), B_Wk.reshape(D * H, Dh), B_Wv.reshape(D * H, Dh),
        B_Wo.reshape(H * Dh, D),
        fwd.astype(BF16), inv.astype(BF16),
    )
    return out.reshape(B, S, 2 * D)
```

```python
import functools

import jax
import jax.numpy as jnp
import numpy as np
from jax import lax
from jax.experimental import pallas as pl
from jax.experimental.pallas import tpu as pltpu

F32 = jnp.float32
BF16 = jnp.bfloat16
U32 = jnp.uint32
LANES = 128
P = 128
AHEAD = 8
XG = 8


def _dft_matrices():
    theta = np.pi * (4 * np.arange(P) + 1) / (2 * P)
    ang = theta[:, None] * np.arange(P)[None, :]
    fwd = np.concatenate([np.cos(ang), -np.sin(ang)], axis=0)
    return fwd.astype(np.float32), (fwd.T / P).astype(np.float32)


def _nn(a, b):
    return lax.dot_general(a, b, (((1,), (0,)), ((), ())), preferred_element_type=F32)


def _nt(a, b):
    return lax.dot_general(a, b, (((1,), (1,)), ((), ())), preferred_element_type=F32)


def _unpacked(words):
    return pltpu.bitcast(words, BF16)


def _packed(x):
    return pltpu.bitcast(x, U32)


def _kernel(
    aq_hbm, ak_hbm, av_hbm, shift_ref, ssmk_hbm, ssmd_ref, x_hbm, mem0_ref,
    wq_hbm, wk_hbm, wv_hbm, wo_hbm, fwd_ref, inv_ref,
    out_hbm,
    aq, ak, av, ssmk, aout, par, kf, kvf, ubuf, kbuf, zbuf,
    raw, wqkv, wo, xa_raw, xa, pre, xs, mem, bout,
    sem_a, sem_w, sem_wo, sem_xa, sem_x, sem_ao, sem_bo,
    *, S, D, H, M, seg,
):
    NB = D // LANES
    Q = S // P
    L = M + seg
    n_seg = S // seg
    KS = shift_ref.shape[0]
    NP = H // 2 // NB
    RG = seg // 8
    SPG = n_seg // XG
    w_hbm = tuple(w.bitcast(U32) for w in (wq_hbm, wk_hbm, wv_hbm))
    wo_words = wo_hbm.bitcast(U32)

    def lane_block(c):
        return pl.ds(pl.multiple_of(c * LANES, LANES), LANES)

    def a_copies(c):
        cols, slot = lane_block(c), c % 2
        return (
            pltpu.make_async_copy(ak_hbm.at[:, cols], ak.at[slot], sem_a.at[slot, 0]),
            pltpu.make_async_copy(av_hbm.at[:, cols], av.at[slot], sem_a.at[slot, 1]),
            pltpu.make_async_copy(ssmk_hbm.at[cols, :], ssmk.at[slot], sem_a.at[slot, 2]),
            pltpu.make_async_copy(aq_hbm.at[:, cols], aq.at[slot], sem_a.at[slot, 3]),
        )

    def w_copies(c):
        slot = c % 2
        return tuple(
            pltpu.make_async_copy(w_hbm[m].at[:, c * NP + i], raw.at[slot, m * NP + i],
                                  sem_w.at[slot, m * NP + i])
            for m in range(3) for i in range(NP)
        )

    def wo_copy(c):
        return pltpu.make_async_copy(wo_words.at[:, lane_block(c)], wo.at[c], sem_wo.at[c])

    def aout_copy(c):
        return pltpu.make_async_copy(aout.at[c], out_hbm.at[:, lane_block(c)], sem_ao.at[c])

    xa_copy = pltpu.make_async_copy(x_hbm.at[:, RG - 1], xa_raw, sem_xa)

    def x_copy(g):
        segs = pl.ds(g * SPG, SPG)
        return pltpu.make_async_copy(
            x_hbm.at[segs, pl.ds(0, RG - 1)], xs.at[segs], sem_x.at[g])

    def bout_copy(g):
        rows = pl.ds(pl.multiple_of(g * SPG * seg, SPG * seg), SPG * seg)
        return pltpu.make_async_copy(
            bout.at[rows, :], out_hbm.at[rows, pl.ds(D, D)], sem_bo.at[g])

    def chunk_conv(p):
        re, im = pl.ds(p * 8, 8), pl.ds(P + p * 8, 8)
        ua = [ubuf[i, re, :] for i in range(Q)]
        ub = [ubuf[i, im, :] for i in range(Q)]
        kc = [kbuf[0, re, :]] + [kbuf[j, re, :] - kbuf[j - 1, im, :] for j in range(1, Q)]
        kd = [kbuf[0, im, :]] + [kbuf[j, im, :] + kbuf[j - 1, re, :] for j in range(1, Q)]
        us = [a + b for a, b in zip(ua, ub)]
        s1 = []
        for a in range(Q):
            t = kc[0] * us[a]
            for j in range(1, a + 1):
                t = t + kc[j] * us[a - j]
            s1.append(t)
        km = [d_ - c_ for c_, d_ in zip(kc, kd)]
        for a in range(Q):
            t = s1[a]
            for j in range(a + 1):
                t = t + km[j] * ua[a - j]
            zbuf[a, im, :] = t
        kp = [d_ + c_ for c_, d_ in zip(kc, kd)]
        for a in range(Q):
            t = s1[a]
            for j in range(a + 1):
                t = t - kp[j] * ub[a - j]
            zbuf[a, re, :] = t

    def project_ahead(c, n):
        pair = raw[c % 2, n]
        head = (n // NP) * H + 2 * (c * NP + n % NP)
        for half, bits in enumerate((pair << 16, pair & np.uint32(0xFFFF0000))):
            w = pltpu.bitcast(bits, F32).astype(BF16)
            wqkv[head + half] = _packed(w)
            pre[head + half] = _nn(_unpacked(xa[...]), w)

    first_a = a_copies(0)
    first_a[0].start()
    first_a[1].start()
    first_a[2].start()
    xa_copy.start()
    for cp in w_copies(0):
        cp.start()
    first_a[3].start()
    kf[pl.ds(0, 8), :] = jnp.zeros((8, LANES), F32)
    shift = shift_ref[...].astype(F32)
    dall = ssmd_ref[...].astype(F32)
    for c in range(NB):
        for j in range(KS):
            par[c, j] = jnp.broadcast_to(shift[j:j + 1, c * LANES:(c + 1) * LANES], (8, LANES))
        par[c, KS] = jnp.broadcast_to(dall[c:c + 1, :], (8, LANES))
    xa_copy.wait()
    xa[...] = _packed(xa_raw[...].astype(F32).reshape(n_seg * AHEAD, D).astype(BF16))

    def stage(c, _):
        @pl.when(c + 1 < NB)
        def _():
            for cp in a_copies(c + 1) + w_copies(c + 1):
                cp.start()

        @pl.when(c + 1 == NB)
        def _():
            x_copy(0).start()

        wo_copy(c).start()
        slot = c % 2
        w = [jnp.tile(par[c, j], (P // 8, 1)) for j in range(KS + 1)]
        for cp in a_copies(c) + w_copies(c):
            cp.wait()

        kf[pl.ds(8, S), :] = ak[slot].astype(F32)
        fwd = fwd_ref[...]
        for j in range(Q):
            kbuf[j] = _nt(fwd, ssmk[slot, :, pl.ds(j * P, P)])
        for i in range(Q):
            acc = kf[pl.ds(8 + i * P - (KS - 1), P), :] * w[KS - 1]
            for j in range(KS - 2, -1, -1):
                acc = acc + kf[pl.ds(8 + i * P - j, P), :] * w[j]
            kv = (acc * av[slot, pl.ds(i * P, P), :].astype(F32)).astype(BF16)
            kvf[pl.ds(i * P, P), :] = kv
            ubuf[i] = _nn(fwd, kv)

        n_pairs, n_pos = 3 * NP, P // 8
        for n in range(n_pairs):
            project_ahead(c, n)
            for p in range(n * n_pos // (n_pairs - 1), (n + 1) * n_pos // (n_pairs - 1)):
                if p < n_pos:
                    chunk_conv(p)

        inv = inv_ref[...]
        for a in range(Q):
            rows = pl.ds(a * P, P)
            y = _nn(inv, zbuf[a].astype(BF16)) + kvf[rows, :].astype(F32) * w[KS]
            aout[c, rows, :] = (aq[slot, rows, :].astype(F32) * y).astype(BF16)
        return 0

    lax.fori_loop(0, NB, stage, 0)
    for c in range(NB):
        wo_copy(c).wait()
    for g in range(1, XG):
        x_copy(g).start()
    for c in range(NB):
        aout_copy(c).start()

    scale = LANES ** -0.5
    row = lax.broadcasted_iota(jnp.int32, (L, L), 0)
    col = lax.broadcasted_iota(jnp.int32, (L, L), 1)
    mask = (row < M) | (row >= col)
    mem[...] = mem0_ref[...].astype(F32)

    def segment(s, _):
        @pl.when(s % SPG == 0)
        def _():
            x_copy(s // SPG).wait()

        rows = pl.ds(pl.multiple_of(s * seg, seg), seg)
        ahead = pl.ds(pl.multiple_of(s * AHEAD, AHEAD), AHEAD)
        h = jnp.concatenate(
            [mem[...], xs[s].astype(F32).reshape(seg - AHEAD, D)], axis=0).astype(BF16)

        def project(i):
            return jnp.concatenate([_nn(h, _unpacked(wqkv[i])), pre[i, ahead, :]], axis=0)

        D1, D2 = 2, 4
        HS = H - 8
        proj, prob, acc, heads = {}, {}, {}, []
        for t in range(H + D2):
            if t < H:
                proj[t] = (project(t), project(H + t).astype(BF16),
                           project(2 * H + t).astype(BF16))
            else:
                for j in range((t - H) * NB // D2, (t - H + 1) * NB // D2):
                    acc[j] = _nn(jnp.concatenate(heads[:HS], axis=1),
                                 _unpacked(wo[j, :HS * LANES // 2, :]))
            if 0 <= t - D1 < H:
                q, k, v = proj.pop(t - D1)
                sc = jnp.where(mask, _nt(q, k) * scale, -1e9)
                e = jnp.exp(sc - jnp.max(sc, axis=-1, keepdims=True))
                prob[t - D1] = (e / jnp.sum(e, axis=-1, keepdims=True), v)
            due = [u for u in prob if u <= (t - D2 if t < H + D2 - 2 else H)]
            for u in due:
                p, v = prob.pop(u)
                heads.append(_nn(p, v))

        for j in range(NB):
            res = _nn(jnp.concatenate(heads[HS:], axis=1),
                      _unpacked(wo[j, HS * LANES // 2:, :])) + acc[j]
            mem[:, pl.ds(j * LANES, LANES)] = res[:M]
            bout[rows, pl.ds(j * LANES, LANES)] = res[M:].astype(BF16)

        @pl.when(s % SPG == SPG - 1)
        def _():
            bout_copy(s // SPG).start()

        return 0

    lax.fori_loop(0, n_seg, segment, 0)
    for c in range(NB):
        aout_copy(c).wait()
    for g in range(XG):
        bout_copy(g).wait()


@functools.partial(jax.jit, static_argnames=("B_seg_len",))
def pallas_concat_heads__ssm_conv_h3__memory_aug_recurrent_mem_tr__prompt_kernel(
    A_q, A_k, A_v, A_shift_k, A_ssm_k, A_ssm_D,
    B_x, B_mem0, B_Wq, B_Wk, B_Wv, B_Wo, B_seg_len,
):
    B, S, D = A_q.shape
    _, H, Dh = B_Wq.shape
    M = B_mem0.shape[1]
    seg = int(B_seg_len)
    assert B == 1 and Dh == LANES and B_x.shape == (B, S, D)
    NB = D // LANES
    Q = S // P
    n_seg = S // seg
    NP = H // 2 // NB
    fwd, inv = _dft_matrices()

    hbm = pl.BlockSpec(memory_space=pl.ANY)
    vmem = pl.BlockSpec(memory_space=pltpu.VMEM)
    out = pl.pallas_call(
        functools.partial(_kernel, S=S, D=D, H=H, M=M, seg=seg),
        out_shape=jax.ShapeDtypeStruct((S, 2 * D), BF16),
        in_specs=[hbm, hbm, hbm, vmem, hbm, vmem, hbm, vmem, hbm, hbm, hbm, hbm, vmem, vmem],
        out_specs=hbm,
        scratch_shapes=[
            pltpu.VMEM((2, S, LANES), BF16),
            pltpu.VMEM((2, S, LANES), BF16),
            pltpu.VMEM((2, S, LANES), BF16),
            pltpu.VMEM((2, LANES, S), BF16),
            pltpu.VMEM((NB, S, LANES), BF16),
            pltpu.VMEM((NB, A_shift_k.shape[1] + 1, 8, LANES), F32),
            pltpu.VMEM((8 + S, LANES), F32),
            pltpu.VMEM((S, LANES), BF16),
            pltpu.VMEM((Q, 2 * P, LANES), F32),
            pltpu.VMEM((Q, 2 * P, LANES), F32),
            pltpu.VMEM((Q, 2 * P, LANES), F32),
            pltpu.VMEM((2, 3 * NP, D, LANES), U32),
            pltpu.VMEM((3 * H, D // 2, LANES), U32),
            pltpu.VMEM((NB, H * Dh // 2, LANES), U32),
            pltpu.VMEM((n_seg, AHEAD, D), BF16),
            pltpu.VMEM((n_seg * AHEAD // 2, D), U32),
            pltpu.VMEM((3 * H, n_seg * AHEAD, LANES), F32),
            pltpu.VMEM((n_seg, seg // 8 - 1, 8, D), BF16),
            pltpu.VMEM((M, D), F32),
            pltpu.VMEM((S, D), BF16),
            pltpu.SemaphoreType.DMA((2, 4)),
            pltpu.SemaphoreType.DMA((2, 3 * NP)),
            pltpu.SemaphoreType.DMA((NB,)),
            pltpu.SemaphoreType.DMA(()),
            pltpu.SemaphoreType.DMA((XG,)),
            pltpu.SemaphoreType.DMA((NB,)),
            pltpu.SemaphoreType.DMA((XG,)),
        ],
        compiler_params=pltpu.CompilerParams(vmem_limit_bytes=120 * 1024 * 1024),
        name="h3_rmt_concat",
    )(
        A_q.reshape(S, D), A_k.reshape(S, D), A_v.reshape(S, D),
        A_shift_k.T, A_ssm_k, A_ssm_D.reshape(NB, LANES),
        B_x.reshape(n_seg, seg // 8, 8, D), B_mem0.reshape(M, D),
        B_Wq, B_Wk, B_Wv, B_Wo.reshape(H * Dh, D),
        fwd.astype(BF16), inv.astype(BF16),
    )
    return out.reshape(B, S, 2 * D)
```

```python
import functools

import jax
import jax.numpy as jnp
import numpy as np
from jax import lax
from jax.experimental import pallas as pl
from jax.experimental.pallas import tpu as pltpu

F32 = jnp.float32
BF16 = jnp.bfloat16
U32 = jnp.uint32
LANES = 128
P = 128
AHEAD = 8
XG = 8
RC = 128
CE = 2
TL = 2
GR = 'pos'
FP = 0.5
UN = 4
KSP = 1


def _dft_matrices():
    theta = np.pi * (4 * np.arange(P) + 1) / (2 * P)
    ang = theta[:, None] * np.arange(P)[None, :]
    fwd = np.concatenate([np.cos(ang), -np.sin(ang)], axis=0)
    return fwd.astype(np.float32), (fwd.T / P).astype(np.float32)


def _nn(a, b):
    return lax.dot_general(a, b, (((1,), (0,)), ((), ())), preferred_element_type=F32)


def _nt(a, b):
    return lax.dot_general(a, b, (((1,), (1,)), ((), ())), preferred_element_type=F32)


def _unpacked(words):
    return pltpu.bitcast(words, BF16)


def _interleave(main, n_main, side, side_total):
    done = 0
    for i, _ in enumerate(main):
        while done < (i + 1) * side_total / n_main:
            step = next(side, None)
            if step is None:
                break
            done += step
    for _ in side:
        pass


def _group(gen, n):
    acc, cnt = 0, 0
    for x in gen:
        acc += x
        cnt += 1
        if cnt == n:
            yield acc
            acc, cnt = 0, 0


def _chain(*gens):
    for g in gens:
        yield from g


def _take(gen, n):
    for _ in range(n):
        yield next(gen)


def _kernel(
    aq_hbm, ak_hbm, av_hbm, shift_hbm, ssmk_hbm, ssmd_hbm, x_hbm, mem0_hbm,
    wq_hbm, wk_hbm, wv_hbm, wo_hbm, fwd_hbm, inv_hbm, base_ref,
    out_hbm,
    shift_ref, ssmd_ref, mem0_ref, fwd_ref, inv_ref,
    aq, ak, av, ssmk, aout, par, kvb, work, raw0, raw, wqkv, wo, xa_raw, xa, xs, bout,
    sem_s, sem_a, sem_w0, sem_w, sem_wo, sem_xa, sem_x, sem_ao, sem_bo,
    *, S, D, H, M, seg,
):
    NB = D // LANES
    Q = S // P
    L = M + seg
    n_seg = S // seg
    NA = n_seg * AHEAD
    KS = shift_ref.shape[0]
    HP = H // 2
    RG = seg // 8
    SPG = n_seg // XG
    w_hbm = tuple(w.bitcast(U32) for w in (wq_hbm, wk_hbm, wv_hbm))
    wqkv_w, wo_w, kvb_w = (r.bitcast(U32) for r in (wqkv, wo, kvb))
    U0 = 3 * H * NA
    K0, Z0, X0 = U0 + 2 * S, U0 + 4 * S, U0 + 6 * S

    def stage_pairs(c):
        return [(0, NB + c * (HP // NB - 1) + i) for i in range(HP // NB - 1)] + [
            (m, c * (HP // NB) + i) for m in (1, 2) for i in range(HP // NB)]

    def lane_block(c):
        return pl.ds(pl.multiple_of(c * LANES, LANES), LANES)

    def stage_copies(c):
        cols, slot = lane_block(c), c % 2
        return [
            pltpu.make_async_copy(ssmk_hbm.at[cols, :], ssmk.at[slot], sem_a.at[slot, 0]),
            pltpu.make_async_copy(ak_hbm.at[:, cols], ak.at[slot], sem_a.at[slot, 1]),
            pltpu.make_async_copy(av_hbm.at[:, cols], av.at[slot], sem_a.at[slot, 2]),
            pltpu.make_async_copy(aq_hbm.at[:, cols], aq.at[slot], sem_a.at[slot, 3]),
        ] + [
            pltpu.make_async_copy(w_hbm[m].at[:, g], raw.at[slot, n], sem_w.at[slot, n])
            for n, (m, g) in enumerate(stage_pairs(c))
        ]

    def first_copy(g):
        return pltpu.make_async_copy(w_hbm[0].at[:, g], raw0.at[g], sem_w0.at[g])

    def wo_copy(c):
        return pltpu.make_async_copy(wo_hbm.at[:, lane_block(c)], wo.at[c], sem_wo.at[c])

    def aout_copy(c):
        return pltpu.make_async_copy(aout.at[c], out_hbm.at[:, lane_block(c)], sem_ao.at[c])

    xa_copy = pltpu.make_async_copy(x_hbm.at[:, RG - 1], xa_raw, sem_xa)

    def x_copy(g):
        segs = pl.ds(g * SPG, SPG)
        return pltpu.make_async_copy(
            x_hbm.at[segs, pl.ds(0, RG - 1)], xs.at[segs], sem_x.at[g])

    def bout_copy(rows):
        return pltpu.make_async_copy(bout.at[rows, :], out_hbm.at[rows, pl.ds(D, D)], sem_bo)

    base = base_ref[0]

    def ordered(offset, size):
        return pl.ds(pl.multiple_of(base + offset, 8), size)

    def split_pair(pair_ref, half, head, piece, pieces):
        rows = pl.ds(piece * D // pieces, D // pieces)
        pair = pair_ref[rows, :]
        bits = pair & np.uint32(0xFFFF0000) if half else pair << 16
        wqkv[head, rows, :] = pltpu.bitcast(bits, F32).astype(BF16)

    def project_ahead(pairs):
        todo = [(ref, half, m * H + 2 * g + half) for ref, m, g in pairs for half in range(2)]
        split_pair(*todo[0], 0, 1)
        yield 0
        for n, (_, _, head) in enumerate(todo):
            for i, r in enumerate(range(0, NA, RC)):
                work[ordered(head * NA + r, RC), :] = _nn(
                    _unpacked(xa[pl.ds(r // 2, RC // 2), :]), _unpacked(wqkv_w[head]))
                if n + 1 < len(todo):
                    split_pair(*todo[n + 1], i, NA // RC)
                yield 1

    def kernel_spectra(slot):
        for j in range(Q):
            work[ordered(K0 + j * 2 * P, 2 * P), :] = _nt(
                fwd_ref[...], ssmk[slot, :, pl.ds(j * P, P)])
            if j % 4 == 3:
                yield 1

    def shift_conv(slot, w):
        for i in range(Q):
            rows = pl.ds(i * P, P)
            k = ak[slot, rows, :].astype(F32)
            work[pl.ds(X0 + 8 + i * P, P), :] = k
            acc = work[pl.ds(X0 + 8 + i * P - (KS - 1), P), :] * w[KS - 1]
            for j in range(KS - 2, 0, -1):
                acc = acc + work[pl.ds(X0 + 8 + i * P - j, P), :] * w[j]
            acc = acc + k * w[0]
            kvb[rows, :] = (acc * av[slot, rows, :].astype(F32)).astype(BF16)
            yield 1

    def chunk_conv():
        for p in range(P // 8):
            def re(b, i):
                return pl.ds(b + i * 2 * P + p * 8, 8)

            def im(b, i):
                return pl.ds(b + i * 2 * P + P + p * 8, 8)

            kc = [work[re(K0, 0), :]] + [
                work[re(K0, j), :] - work[im(K0, j - 1), :] for j in range(1, Q)]
            us = [work[re(U0, i), :] + work[im(U0, i), :] for i in range(Q)]
            yield 2 * Q
            s1 = []
            for a in range(Q):
                t = kc[0] * us[a]
                for j in range(1, a + 1):
                    t = t + kc[j] * us[a - j]
                s1.append(t)
                yield 2 * (a + 1)
            kd = [work[im(K0, 0), :]] + [
                work[im(K0, j), :] + work[re(K0, j - 1), :] for j in range(1, Q)]
            km = [d_ - c_ for c_, d_ in zip(kc, kd)]
            kp = [d_ + c_ for c_, d_ in zip(kc, kd)]
            yield 3 * Q
            ua = [work[re(U0, i), :] for i in range(Q)]
            for a in range(Q):
                t = s1[a]
                for j in range(a + 1):
                    t = t + km[j] * ua[a - j]
                work[im(Z0, a), :] = t
                yield 2 * (a + 1)
            ub = [work[im(U0, i), :] for i in range(Q)]
            for a in range(Q):
                t = s1[a]
                for j in range(a + 1):
                    t = t - kp[j] * ub[a - j]
                work[re(Z0, a), :] = t
                yield 2 * (a + 1)

    small = [
        pltpu.make_async_copy(src, dst, sem_s.at[i]) for i, (src, dst) in enumerate(zip(
            (shift_hbm, ssmd_hbm, mem0_hbm, fwd_hbm, inv_hbm),
            (shift_ref, ssmd_ref, mem0_ref, fwd_ref, inv_ref)))
    ]
    xa_copy.start()
    for cp in small:
        cp.start(priority=1)
    small[0].wait()
    small[1].wait()
    work[pl.ds(X0, 8), :] = jnp.zeros((8, LANES), F32)
    shift = shift_ref[...].astype(F32)
    dall = ssmd_ref[...].astype(F32)
    for c in range(NB):
        for j in range(KS):
            par[c, j] = jnp.broadcast_to(shift[j:j + 1, c * LANES:(c + 1) * LANES], (8, LANES))
        par[c, KS] = jnp.broadcast_to(dall[c:c + 1, :], (8, LANES))
    for cp in small[2:]:
        cp.wait()
    for g in range(NB):
        first_copy(g).start()
    xa_copy.wait()
    for cp in stage_copies(0):
        cp.start()
    xa[...] = pltpu.bitcast(xa_raw[...].astype(F32).reshape(NA, D).astype(BF16), U32)

    def warm_up(g, _):
        first_copy(g).wait()
        for _ in project_ahead([(raw0.at[g], 0, g)]):
            pass
        return 0

    lax.fori_loop(0, NB, warm_up, 0)

    def stage(c, _):
        @pl.when(c + 1 < NB)
        def _():
            for cp in stage_copies(c + 1):
                cp.start()

        @pl.when(c + 1 == NB)
        def _():
            x_copy(0).start()

        wo_copy(c).start()
        for cp in stage_copies(c):
            cp.wait()
        slot = c % 2
        w = [jnp.tile(par[c, j], (P // 8, 1)) for j in range(KS + 1)]
        pairs = stage_pairs(c)
        ahead = project_ahead([(raw.at[slot, n], m, g) for n, (m, g) in enumerate(pairs)])
        next(ahead)
        per_pair = 2 * NA // RC
        tail = TL

        _interleave(_chain(kernel_spectra(slot), _take(ahead, int(FP * per_pair))), Q // 4 + int(FP * per_pair) - 1,
                    shift_conv(slot, w), Q)
        for i in range(Q):
            work[ordered(U0 + i * 2 * P, 2 * P), :] = _nn(
                fwd_ref[...], _unpacked(kvb_w[pl.ds(i * P // 2, P // 2), :]))
        _interleave(_take(ahead, len(pairs) * per_pair - int(FP * per_pair) - tail), CE * per_pair,
                    _group(chunk_conv(), {'a': 1, 'pos': 3 * Q + 2, 'half': (3 * Q + 2) // 2}[GR]), P // 8 * (5 * Q + 3 * Q * (Q + 1)))
        for a in range(Q):
            rows = pl.ds(a * P, P)
            kv = _unpacked(kvb_w[pl.ds(a * P // 2, P // 2), :]).astype(F32)
            z = work[pl.ds(Z0 + a * 2 * P, 2 * P), :].astype(BF16)
            y = _nn(inv_ref[...], z) + kv * w[KS]
            aout[c, rows, :] = (aq[slot, rows, :].astype(F32) * y).astype(BF16)
        for _ in ahead:
            pass
        return 0

    lax.fori_loop(0, NB, stage, 0)
    for c in range(NB):
        wo_copy(c).wait()
    for g in range(1, XG):
        x_copy(g).start()
    for c in range(NB):
        aout_copy(c).start()

    scale = LANES ** -0.5
    row = lax.broadcasted_iota(jnp.int32, (L, L), 0)
    col = lax.broadcasted_iota(jnp.int32, (L, L), 1)
    mask = (row < M) | (row >= col)

    def segment(s, state):
        rows = pl.ds(pl.multiple_of(s * seg, seg), seg)
        h = jnp.concatenate(
            [state, xs[s].astype(F32).reshape(seg - AHEAD, D)], axis=0).astype(BF16)

        def finish(i, late):
            early = work[pl.ds(pl.multiple_of(i * NA + s * AHEAD, AHEAD), AHEAD), :]
            return jnp.concatenate([late, early], axis=0)

        D1, D2 = 2, 4
        HS = H - 8
        proj, prob, acc, heads = {}, {}, {}, []
        for t in range(H + D2):
            if t < H:
                ids = [m * H + t for m in range(3)]
                if t == 0 and KSP:
                    lo = [_nn(h[:, :D // 2], _unpacked(wqkv_w[i, :D // 4, :])) for i in ids]
                    late = [_nn(h[:, D // 2:], _unpacked(wqkv_w[i, D // 4:, :])) + part
                            for i, part in zip(ids, lo)]
                else:
                    late = [_nn(h, _unpacked(wqkv_w[i])) for i in ids]
                q, k, v = (finish(i, y) for i, y in zip(ids, late))
                proj[t] = (q, k.astype(BF16), v.astype(BF16))
            else:
                for j in range((t - H) * NB // D2, (t - H + 1) * NB // D2):
                    acc[j] = _nn(jnp.concatenate(heads[:HS], axis=1),
                                 _unpacked(wo_w[j, :HS * LANES // 2, :]))
            if 0 <= t - D1 < H:
                q, k, v = proj.pop(t - D1)
                sc = jnp.where(mask, _nt(q, k) * scale, -1e9)
                e = jnp.exp(sc - jnp.max(sc, axis=-1, keepdims=True))
                prob[t - D1] = (e / jnp.sum(e, axis=-1, keepdims=True), v)
            due = [u for u in prob if u <= (t - D2 if t < H + D2 - 2 else H)]
            for u in due:
                p, v = prob.pop(u)
                heads.append(_nn(p, v))

        new_state = []
        for j in range(NB):
            res = _nn(jnp.concatenate(heads[HS:], axis=1),
                      _unpacked(wo_w[j, HS * LANES // 2:, :])) + acc[j]
            new_state.append(res[:M])
            bout[rows, pl.ds(j * LANES, LANES)] = res[M:].astype(BF16)
        return jnp.concatenate(new_state, axis=1)

    def segments(i, state):
        @pl.when(i % (SPG // UN) == 0)
        def _():
            x_copy(i // (SPG // UN)).wait()

        for u in range(UN):
            state = segment(i * UN + u, state)
        bout_copy(pl.ds(pl.multiple_of(i * UN * seg, UN * seg), UN * seg)).start()
        return state

    lax.fori_loop(0, n_seg // UN, segments, mem0_ref[...].astype(F32))
    for c in range(NB):
        aout_copy(c).wait()
    bout_copy(pl.ds(0, S)).wait()


@functools.partial(jax.jit, static_argnames=("B_seg_len",))
def pallas_concat_heads__ssm_conv_h3__memory_aug_recurrent_mem_tr__prompt_kernel(
    A_q, A_k, A_v, A_shift_k, A_ssm_k, A_ssm_D,
    B_x, B_mem0, B_Wq, B_Wk, B_Wv, B_Wo, B_seg_len,
):
    B, S, D = A_q.shape
    _, H, Dh = B_Wq.shape
    M = B_mem0.shape[1]
    seg = int(B_seg_len)
    assert B == 1 and Dh == LANES and B_x.shape == (B, S, D)
    NB = D // LANES
    n_seg = S // seg
    NA = n_seg * AHEAD
    n_pairs = 3 * (H // 2) // NB - 1
    fwd, inv = _dft_matrices()

    hbm = pl.BlockSpec(memory_space=pl.ANY)
    vmem = pl.BlockSpec(memory_space=pltpu.VMEM)
    smem = pl.BlockSpec(memory_space=pltpu.SMEM)
    out = pl.pallas_call(
        functools.partial(_kernel, S=S, D=D, H=H, M=M, seg=seg),
        out_shape=jax.ShapeDtypeStruct((S, 2 * D), BF16),
        in_specs=[hbm] * 14 + [smem],
        out_specs=hbm,
        scratch_shapes=[
            pltpu.VMEM(A_shift_k.shape[::-1], BF16),
            pltpu.VMEM((NB, LANES), BF16),
            pltpu.VMEM((M, D), BF16),
            pltpu.VMEM(fwd.shape, BF16),
            pltpu.VMEM(inv.shape, BF16),
            pltpu.VMEM((2, S, LANES), BF16),
            pltpu.VMEM((2, S, LANES), BF16),
            pltpu.VMEM((2, S, LANES), BF16),
            pltpu.VMEM((2, LANES, S), BF16),
            pltpu.VMEM((NB, S, LANES), BF16),
            pltpu.VMEM((NB, A_shift_k.shape[1] + 1, 8, LANES), F32),
            pltpu.VMEM((S, LANES), BF16),
            pltpu.VMEM((3 * H * NA + 7 * S + 8, LANES), F32),
            pltpu.VMEM((NB, D, LANES), U32),
            pltpu.VMEM((2, n_pairs, D, LANES), U32),
            pltpu.VMEM((3 * H, D, LANES), BF16),
            pltpu.VMEM((NB, H * Dh, LANES), BF16),
            pltpu.VMEM((n_seg, AHEAD, D), BF16),
            pltpu.VMEM((NA // 2, D), U32),
            pltpu.VMEM((n_seg, seg // 8 - 1, 8, D), BF16),
            pltpu.VMEM((S, D), BF16),
            pltpu.SemaphoreType.DMA((5,)),
            pltpu.SemaphoreType.DMA((2, 4)),
            pltpu.SemaphoreType.DMA((NB,)),
            pltpu.SemaphoreType.DMA((2, n_pairs)),
            pltpu.SemaphoreType.DMA((NB,)),
            pltpu.SemaphoreType.DMA(()),
            pltpu.SemaphoreType.DMA((XG,)),
            pltpu.SemaphoreType.DMA((NB,)),
            pltpu.SemaphoreType.DMA(()),
        ],
        compiler_params=pltpu.CompilerParams(vmem_limit_bytes=120 * 1024 * 1024),
        name="h3_rmt_concat",
    )(
        A_q.reshape(S, D), A_k.reshape(S, D), A_v.reshape(S, D),
        A_shift_k.T, A_ssm_k, A_ssm_D.reshape(NB, LANES),
        B_x.reshape(n_seg, seg // 8, 8, D), B_mem0.reshape(M, D),
        B_Wq, B_Wk, B_Wv, B_Wo.reshape(H * Dh, D),
        fwd.astype(BF16), inv.astype(BF16), np.zeros((1,), np.int32),
    )
    return out.reshape(B, S, 2 * D)
```

```python
import functools

import jax
import jax.numpy as jnp
import numpy as np
from jax import lax
from jax.experimental import pallas as pl
from jax.experimental.pallas import tpu as pltpu

F32 = jnp.float32
BF16 = jnp.bfloat16
U32 = jnp.uint32
LANES = 128
P = 128
PITCH = 2 * P + 8
AHEAD = 8
XG = 8
UNROLL = 4


def _dft_matrices():
    theta = np.pi * (4 * np.arange(P) + 1) / (2 * P)
    ang = theta[:, None] * np.arange(P)[None, :]
    fwd = np.concatenate([np.cos(ang), -np.sin(ang)], axis=0)
    return fwd.astype(BF16), (fwd.T / P).astype(BF16)


def _nn(a, b):
    return lax.dot_general(a, b, (((1,), (0,)), ((), ())), preferred_element_type=F32)


def _nt(a, b):
    return lax.dot_general(a, b, (((1,), (1,)), ((), ())), preferred_element_type=F32)


def _unpacked(words):
    return pltpu.bitcast(words, BF16)


def _interleave(main, n_main, side, side_total):
    done = 0
    for i, _ in enumerate(main):
        while done < (i + 1) * side_total / n_main:
            step = next(side, None)
            if step is None:
                break
            done += step
    for _ in side:
        pass


def _chain(*gens):
    for g in gens:
        yield from g


def _take(gen, n):
    for _ in range(n):
        yield next(gen)


def _kernel(
    aq_hbm, ak_hbm, av_hbm, shift_hbm, ssmk_hbm, ssmd_hbm, x_hbm, mem0_hbm,
    wq_hbm, wk_hbm, wv_hbm, wo_hbm, fwd_hbm, inv_hbm, base_ref,
    out_hbm,
    shift_ref, ssmd_ref, mem0_ref, fwd_ref, inv_ref,
    aq, ak, av, ssmk, aout, par, kvb, work, raw0, raw, wqkv, wo, xa_raw, xa, xs, bout,
    sem_s, sem_a, sem_w0, sem_w, sem_wo, sem_xa, sem_x, sem_ao, sem_bo,
    *, S, D, H, M, seg,
):
    NB = D // LANES
    Q = S // P
    L = M + seg
    n_seg = S // seg
    NA = n_seg * AHEAD
    KS = shift_ref.shape[0]
    PPS = H // 2 // NB
    RG = seg // AHEAD
    SPG = n_seg // XG
    w_hbm = tuple(w.bitcast(U32) for w in (wq_hbm, wk_hbm, wv_hbm))
    wqkv_w, wo_w, kvb_w, fwd_w, aq_w, ak_w, av_w = (
        r.bitcast(U32) for r in (wqkv, wo, kvb, fwd_ref, aq, ak, av))
    U0 = 3 * H * NA
    K0, Z0, X0 = (U0 + i * Q * PITCH for i in (1, 2, 3))

    def stage_pairs(c):
        return [(0, NB + c * (PPS - 1) + i) for i in range(PPS - 1)] + [
            (m, c * PPS + i) for m in (1, 2) for i in range(PPS)]

    def lane_block(c):
        return pl.ds(pl.multiple_of(c * LANES, LANES), LANES)

    def stage_copies(c):
        cols, slot = lane_block(c), c % 2
        return [
            pltpu.make_async_copy(ssmk_hbm.at[cols, :], ssmk.at[slot], sem_a.at[slot, 0]),
            pltpu.make_async_copy(ak_hbm.at[:, cols], ak.at[slot], sem_a.at[slot, 1]),
            pltpu.make_async_copy(av_hbm.at[:, cols], av.at[slot], sem_a.at[slot, 2]),
            pltpu.make_async_copy(aq_hbm.at[:, cols], aq.at[slot], sem_a.at[slot, 3]),
        ] + [
            pltpu.make_async_copy(w_hbm[m].at[:, g], raw.at[slot, n], sem_w.at[slot, n])
            for n, (m, g) in enumerate(stage_pairs(c))
        ]

    def first_copy(g):
        return pltpu.make_async_copy(w_hbm[0].at[:, g], raw0.at[g], sem_w0.at[g])

    def wo_copy(c):
        return pltpu.make_async_copy(wo_hbm.at[:, lane_block(c)], wo.at[c], sem_wo.at[c])

    def aout_copy(c):
        return pltpu.make_async_copy(aout.at[c], out_hbm.at[:, lane_block(c)], sem_ao.at[c])

    def x_copy(g):
        segs = pl.ds(g * SPG, SPG)
        return pltpu.make_async_copy(
            x_hbm.at[segs, pl.ds(0, RG - 1)], xs.at[segs], sem_x.at[g])

    def bout_copy(rows):
        return pltpu.make_async_copy(bout.at[rows, :], out_hbm.at[rows, pl.ds(D, D)], sem_bo)

    base = base_ref[0]

    def ordered(offset, size):
        return pl.ds(pl.multiple_of(base + offset, 8), size)

    def split_pair(pair_ref, half, head, piece, pieces):
        rows = pl.ds(piece * D // pieces, D // pieces)
        pair = pair_ref[rows, :]
        bits = pair & np.uint32(0xFFFF0000) if half else pair << 16
        wqkv[head, rows, :] = pltpu.bitcast(bits, F32).astype(BF16)

    def project_ahead(pairs, step):
        todo = [(ref, half, m * H + 2 * g + half) for ref, m, g in pairs for half in range(2)]
        split_pair(*todo[0], 0, 1)
        yield
        for n, (_, _, head) in enumerate(todo):
            for r in range(0, NA, step):
                work[ordered(head * NA + r, step), :] = _nn(
                    _unpacked(xa[pl.ds(r // 2, step // 2), :]), _unpacked(wqkv_w[head]))
                if n + 1 < len(todo):
                    split_pair(*todo[n + 1], r // step, NA // step)
                yield

    def kernel_spectra(slot):
        for j in range(Q):
            work[ordered(K0 + j * PITCH, 2 * P), :] = _nt(
                _unpacked(fwd_w[...]), ssmk[slot, :, pl.ds(j * P, P)])
            if j % 4 == 3:
                yield

    def shift_conv(c, step):
        for r in range(0, S, step):
            w = [jnp.tile(par[c, j], (step // 8, 1)) for j in range(KS)]
            words = pl.ds(r // 2, step // 2)
            k = _unpacked(ak_w[c % 2, words, :]).astype(F32)
            work[pl.ds(X0 + 8 + r, step), :] = k
            acc = work[pl.ds(X0 + 8 + r - (KS - 1), step), :] * w[KS - 1]
            for j in range(KS - 2, 0, -1):
                acc = acc + work[pl.ds(X0 + 8 + r - j, step), :] * w[j]
            acc = acc + k * w[0]
            v = _unpacked(av_w[c % 2, words, :]).astype(F32)
            kvb[pl.ds(r, step), :] = (acc * v).astype(BF16)
            yield 1

    def chunk_conv():
        for f in range(0, P, 8):
            def re(b, i):
                return pl.ds(b + i * PITCH + f, 8)

            def im(b, i):
                return pl.ds(b + i * PITCH + P + f, 8)

            kc = [work[re(K0, 0), :]] + [
                work[re(K0, j), :] - work[im(K0, j - 1), :] for j in range(1, Q)]
            us = [work[re(U0, i), :] + work[im(U0, i), :] for i in range(Q)]
            yield 2 * Q
            s1 = []
            for a in range(Q):
                t = kc[0] * us[a]
                for j in range(1, a + 1):
                    t = t + kc[j] * us[a - j]
                s1.append(t)
                yield 2 * (a + 1)
            kd = [work[im(K0, 0), :]] + [
                work[im(K0, j), :] + work[re(K0, j - 1), :] for j in range(1, Q)]
            km = [d_ - c_ for c_, d_ in zip(kc, kd)]
            kp = [d_ + c_ for c_, d_ in zip(kc, kd)]
            yield 3 * Q
            ua = [work[re(U0, i), :] for i in range(Q)]
            for a in range(Q):
                t = s1[a]
                for j in range(a + 1):
                    t = t + km[j] * ua[a - j]
                work[im(Z0, a), :] = t
                yield 2 * (a + 1)
            ub = [work[im(U0, i), :] for i in range(Q)]
            for a in range(Q):
                t = s1[a]
                for j in range(a + 1):
                    t = t - kp[j] * ub[a - j]
                work[re(Z0, a), :] = t
                yield 2 * (a + 1)

    xa_copy = pltpu.make_async_copy(x_hbm.at[:, RG - 1], xa_raw, sem_xa)
    small = [
        pltpu.make_async_copy(src, dst, sem_s.at[i]) for i, (src, dst) in enumerate(zip(
            (shift_hbm, ssmd_hbm, mem0_hbm, fwd_hbm, inv_hbm),
            (shift_ref, ssmd_ref, mem0_ref, fwd_ref, inv_ref)))
    ]
    small[0].start()
    small[1].start()
    first_copy(0).start()
    xa_copy.start()
    small[0].wait()
    small[1].wait()
    for g in range(1, NB):
        first_copy(g).start()
    work[pl.ds(X0, 8), :] = jnp.zeros((8, LANES), F32)
    shift = shift_ref[...].astype(F32)
    skip_all = ssmd_ref[...].astype(F32)
    for c in range(NB):
        for j in range(KS):
            par[c, j] = jnp.broadcast_to(shift[j:j + 1, c * LANES:(c + 1) * LANES], (8, LANES))
        par[c, KS] = jnp.broadcast_to(skip_all[c:c + 1, :], (8, LANES))
    xa_copy.wait()
    for cp in small[2:] + stage_copies(0):
        cp.start()
    xa[...] = pltpu.bitcast(xa_raw[...].astype(F32).reshape(NA, D).astype(BF16), U32)

    def warm_up(g, _):
        first_copy(g).wait()
        for _ in project_ahead([(raw0.at[g], 0, g)], 128):
            pass
        return 0

    lax.fori_loop(0, NB, warm_up, 0)
    for cp in small[2:]:
        cp.wait()

    def stage(c, _):
        @pl.when(c + 1 < NB)
        def _():
            for cp in stage_copies(c + 1):
                cp.start()

        @pl.when(c + 1 == NB)
        def _():
            x_copy(0).start()

        wo_copy(c).start()
        for cp in stage_copies(c):
            cp.wait()
        slot = c % 2
        pairs = stage_pairs(c)
        ahead = project_ahead(
            [(raw.at[slot, n], m, g) for n, (m, g) in enumerate(pairs)], 64)
        next(ahead)
        per_pair = 2 * NA // 64

        _interleave(_chain(kernel_spectra(slot), _take(ahead, per_pair)), per_pair,
                    shift_conv(c, 32), S // 32)
        for i in range(Q):
            work[ordered(U0 + i * PITCH, 2 * P), :] = _nn(
                _unpacked(fwd_w[...]), _unpacked(kvb_w[pl.ds(i * P // 2, P // 2), :]))
        _interleave(_take(ahead, (len(pairs) - 1) * per_pair - 2), 1.75 * per_pair,
                    chunk_conv(), P // 8 * (5 * Q + 3 * Q * (Q + 1)))
        skip = jnp.tile(par[c, KS], (P // 8, 1))
        for a in range(Q):
            words = pl.ds(a * P // 2, P // 2)
            z = work[pl.ds(Z0 + a * PITCH, 2 * P), :].astype(BF16)
            y = _nn(inv_ref[...], z) + _unpacked(kvb_w[words, :]).astype(F32) * skip
            q = _unpacked(aq_w[slot, words, :]).astype(F32)
            aout[c, pl.ds(a * P, P), :] = (q * y).astype(BF16)
        for _ in ahead:
            pass
        return 0

    lax.fori_loop(0, NB, stage, 0)
    for c in range(NB):
        wo_copy(c).wait()
    for g in range(1, XG):
        x_copy(g).start()
    for c in range(NB):
        aout_copy(c).start()

    scale = LANES ** -0.5
    row = lax.broadcasted_iota(jnp.int32, (L, L), 0)
    col = lax.broadcasted_iota(jnp.int32, (L, L), 1)
    mask = (row < M) | (row >= col)

    def segment(s, mem):
        rows = pl.ds(pl.multiple_of(s * seg, seg), seg)
        h = jnp.concatenate(
            [mem, xs[s].astype(F32).reshape(seg - AHEAD, D)], axis=0).astype(BF16)

        def finish(i, late):
            early = work[pl.ds(pl.multiple_of(i * NA + s * AHEAD, AHEAD), AHEAD), :]
            return jnp.concatenate([late, early], axis=0)

        D1, D2 = 2, 4
        HS = H - 8
        proj, prob, acc, heads = {}, {}, {}, []
        for t in range(H + D2):
            if t < H:
                ids = [m * H + t for m in range(3)]
                if t == 0:
                    lo = [_nn(h[:, :D // 2], _unpacked(wqkv_w[i, :D // 4, :])) for i in ids]
                    late = [_nn(h[:, D // 2:], _unpacked(wqkv_w[i, D // 4:, :])) + part
                            for i, part in zip(ids, lo)]
                else:
                    late = [_nn(h, _unpacked(wqkv_w[i])) for i in ids]
                q, k, v = (finish(i, y) for i, y in zip(ids, late))
                proj[t] = (q, k.astype(BF16), v.astype(BF16))
            else:
                for j in range((t - H) * NB // D2, (t - H + 1) * NB // D2):
                    acc[j] = _nn(jnp.concatenate(heads[:HS], axis=1),
                                 _unpacked(wo_w[j, :HS * LANES // 2, :]))
            if 0 <= t - D1 < H:
                q, k, v = proj.pop(t - D1)
                sc = jnp.where(mask, _nt(q, k) * scale, -1e9)
                e = jnp.exp(sc - jnp.max(sc, axis=-1, keepdims=True))
                den = jnp.sum(e, axis=-1, keepdims=True)
                prob[t - D1] = (e * pltpu.reciprocal(den, approx=False, full_range=False), v)
            for u in [u for u in prob if u <= (t - D2 if t < H + D2 - 2 else H)]:
                p, v = prob.pop(u)
                heads.append(_nn(p, v))

        new_mem = []
        for j in range(NB):
            res = _nn(jnp.concatenate(heads[HS:], axis=1),
                      _unpacked(wo_w[j, HS * LANES // 2:, :])) + acc[j]
            new_mem.append(res[:M])
            bout[rows, pl.ds(j * LANES, LANES)] = res[M:].astype(BF16)
        bout_copy(rows).start()
        return jnp.concatenate(new_mem, axis=1)

    def segments(i, mem):
        @pl.when(i % (SPG // UNROLL) == 0)
        def _():
            x_copy(i // (SPG // UNROLL)).wait()

        for u in range(UNROLL):
            mem = segment(i * UNROLL + u, mem)
        return mem

    lax.fori_loop(0, n_seg // UNROLL, segments, mem0_ref[...].astype(F32))
    for c in range(NB):
        aout_copy(c).wait()
    bout_copy(pl.ds(0, S)).wait()


@functools.partial(jax.jit, static_argnames=("B_seg_len",))
def pallas_concat_heads__ssm_conv_h3__memory_aug_recurrent_mem_tr__prompt_kernel(
    A_q, A_k, A_v, A_shift_k, A_ssm_k, A_ssm_D,
    B_x, B_mem0, B_Wq, B_Wk, B_Wv, B_Wo, B_seg_len,
):
    B, S, D = A_q.shape
    _, H, Dh = B_Wq.shape
    M = B_mem0.shape[1]
    KS = A_shift_k.shape[1]
    seg = int(B_seg_len)
    assert B == 1 and Dh == LANES and B_x.shape == (B, S, D)
    NB = D // LANES
    n_seg = S // seg
    NA = n_seg * AHEAD
    n_pairs = 3 * (H // 2 // NB) - 1
    fwd, inv = _dft_matrices()

    hbm = pl.BlockSpec(memory_space=pl.ANY)
    out = pl.pallas_call(
        functools.partial(_kernel, S=S, D=D, H=H, M=M, seg=seg),
        out_shape=jax.ShapeDtypeStruct((S, 2 * D), BF16),
        in_specs=[hbm] * 14 + [pl.BlockSpec(memory_space=pltpu.SMEM)],
        out_specs=hbm,
        scratch_shapes=[
            pltpu.VMEM((KS, D), BF16),
            pltpu.VMEM((NB, LANES), BF16),
            pltpu.VMEM((M, D), BF16),
            pltpu.VMEM(fwd.shape, BF16),
            pltpu.VMEM(inv.shape, BF16),
            pltpu.VMEM((2, S, LANES), BF16),
            pltpu.VMEM((2, S, LANES), BF16),
            pltpu.VMEM((2, S, LANES), BF16),
            pltpu.VMEM((2, LANES, S), BF16),
            pltpu.VMEM((NB, S, LANES), BF16),
            pltpu.VMEM((NB, KS + 1, 8, LANES), F32),
            pltpu.VMEM((S, LANES), BF16),
            pltpu.VMEM((3 * H * NA + 3 * (S // P) * PITCH + 8 + S, LANES), F32),
            pltpu.VMEM((NB, D, LANES), U32),
            pltpu.VMEM((2, n_pairs, D, LANES), U32),
            pltpu.VMEM((3 * H, D, LANES), BF16),
            pltpu.VMEM((NB, H * Dh, LANES), BF16),
            pltpu.VMEM((n_seg, AHEAD, D), BF16),
            pltpu.VMEM((NA // 2, D), U32),
            pltpu.VMEM((n_seg, seg // AHEAD - 1, AHEAD, D), BF16),
            pltpu.VMEM((S, D), BF16),
            pltpu.SemaphoreType.DMA((5,)),
            pltpu.SemaphoreType.DMA((2, 4)),
            pltpu.SemaphoreType.DMA((NB,)),
            pltpu.SemaphoreType.DMA((2, n_pairs)),
            pltpu.SemaphoreType.DMA((NB,)),
            pltpu.SemaphoreType.DMA(()),
            pltpu.SemaphoreType.DMA((XG,)),
            pltpu.SemaphoreType.DMA((NB,)),
            pltpu.SemaphoreType.DMA(()),
        ],
        compiler_params=pltpu.CompilerParams(
            vmem_limit_bytes=112 * 1024 * 1024, disable_bounds_checks=True),
        name="h3_rmt_concat",
    )(
        A_q.reshape(S, D), A_k.reshape(S, D), A_v.reshape(S, D),
        A_shift_k.T, A_ssm_k, A_ssm_D.reshape(NB, LANES),
        B_x.reshape(n_seg, seg // AHEAD, AHEAD, D), B_mem0.reshape(M, D),
        B_Wq, B_Wk, B_Wv, B_Wo.reshape(H * Dh, D),
        fwd, inv, np.zeros((1,), np.int32),
    )
    return out.reshape(B, S, 2 * D)
```

```python
import functools

import jax
import jax.numpy as jnp
import numpy as np
from jax import lax
from jax.experimental import pallas as pl
from jax.experimental.pallas import tpu as pltpu

F32 = jnp.float32
BF16 = jnp.bfloat16
U32 = jnp.uint32
LANES = 128
P = 128
PITCH = 2 * P + 8
AHEAD = 8
XG = 8
UNROLL = 4


def _dft_matrices():
    theta = np.pi * (4 * np.arange(P) + 1) / (2 * P)
    ang = theta[:, None] * np.arange(P)[None, :]
    fwd = np.concatenate([np.cos(ang), -np.sin(ang)], axis=0)
    return fwd.astype(BF16), (fwd.T / P).astype(BF16)


def _nn(a, b):
    return lax.dot_general(a, b, (((1,), (0,)), ((), ())), preferred_element_type=F32)


def _nt(a, b):
    return lax.dot_general(a, b, (((1,), (1,)), ((), ())), preferred_element_type=F32)


def _unpacked(words):
    return pltpu.bitcast(words, BF16)


def _interleave(main, n_main, side, side_total):
    done = 0
    for i, _ in enumerate(main):
        while done < (i + 1) * side_total / n_main:
            step = next(side, None)
            if step is None:
                break
            done += step
    for _ in side:
        pass


def _chain(*gens):
    for g in gens:
        yield from g


def _take(gen, n):
    for _ in range(n):
        yield next(gen)


def _kernel(
    aq_hbm, ak_hbm, av_hbm, shift_hbm, ssmk_hbm, ssmd_hbm, x_hbm, mem0_hbm,
    wq_hbm, wk_hbm, wv_hbm, wo_hbm, fwd_hbm, inv_hbm, base_ref,
    out_hbm,
    shift_ref, ssmd_ref, mem0_ref, fwd_ref, inv_ref,
    aq, ak, av, ssmk, aout, par, kvb, work, raw0, raw, wqkv, wo, xa_raw, xa, xs, bout,
    sem_s, sem_a, sem_w0, sem_w, sem_wo, sem_xa, sem_x, sem_ao, sem_bo,
    *, S, D, H, M, seg,
):
    NB = D // LANES
    Q = S // P
    L = M + seg
    n_seg = S // seg
    NA = n_seg * AHEAD
    KS = shift_ref.shape[0]
    PPS = H // 2 // NB
    RG = seg // AHEAD
    SPG = n_seg // XG
    w_hbm = tuple(w.bitcast(U32) for w in (wq_hbm, wk_hbm, wv_hbm))
    wqkv_w, wo_w, kvb_w, fwd_w, aq_w, ak_w, av_w = (
        r.bitcast(U32) for r in (wqkv, wo, kvb, fwd_ref, aq, ak, av))
    U0 = 3 * H * NA
    K0, Z0, X0 = (U0 + i * Q * PITCH for i in (1, 2, 3))

    def stage_pairs(c):
        return [(0, NB + c * (PPS - 1) + i) for i in range(PPS - 1)] + [
            (m, c * PPS + i) for m in (1, 2) for i in range(PPS)]

    def lane_block(c):
        return pl.ds(pl.multiple_of(c * LANES, LANES), LANES)

    def stage_copies(c):
        cols, slot = lane_block(c), c % 2
        return [
            pltpu.make_async_copy(ssmk_hbm.at[cols, :], ssmk.at[slot], sem_a.at[slot, 0]),
            pltpu.make_async_copy(ak_hbm.at[:, cols], ak.at[slot], sem_a.at[slot, 1]),
            pltpu.make_async_copy(av_hbm.at[:, cols], av.at[slot], sem_a.at[slot, 2]),
            pltpu.make_async_copy(aq_hbm.at[:, cols], aq.at[slot], sem_a.at[slot, 3]),
        ] + [
            pltpu.make_async_copy(w_hbm[m].at[:, g], raw.at[slot, n], sem_w.at[slot, n])
            for n, (m, g) in enumerate(stage_pairs(c))
        ]

    def first_copy(g):
        return pltpu.make_async_copy(w_hbm[0].at[:, g], raw0.at[g], sem_w0.at[g])

    def wo_copy(c):
        return pltpu.make_async_copy(wo_hbm.at[:, lane_block(c)], wo.at[c], sem_wo.at[c])

    def aout_copy(c):
        return pltpu.make_async_copy(aout.at[c], out_hbm.at[:, lane_block(c)], sem_ao.at[c])

    def x_copy(g):
        segs = pl.ds(g * SPG, SPG)
        return pltpu.make_async_copy(
            x_hbm.at[segs, pl.ds(0, RG - 1)], xs.at[segs], sem_x.at[g])

    def bout_copy(rows):
        return pltpu.make_async_copy(bout.at[rows, :], out_hbm.at[rows, pl.ds(D, D)], sem_bo)

    base = base_ref[0]

    def ordered(offset, size):
        return pl.ds(pl.multiple_of(base + offset, 8), size)

    def split_pair(pair_ref, half, head, piece, pieces):
        rows = pl.ds(piece * D // pieces, D // pieces)
        pair = pair_ref[rows, :]
        bits = pair & np.uint32(0xFFFF0000) if half else pair << 16
        wqkv[head, rows, :] = pltpu.bitcast(bits, F32).astype(BF16)

    def project_ahead(pairs, step):
        todo = [(ref, half, m * H + 2 * g + half) for ref, m, g in pairs for half in range(2)]
        split_pair(*todo[0], 0, 1)
        yield
        for n, (_, _, head) in enumerate(todo):
            for r in range(0, NA, step):
                work[ordered(head * NA + r, step), :] = _nn(
                    _unpacked(xa[pl.ds(r // 2, step // 2), :]), _unpacked(wqkv_w[head]))
                if n + 1 < len(todo):
                    split_pair(*todo[n + 1], r // step, NA // step)
                yield

    def kernel_spectra(slot):
        for j in range(Q):
            work[ordered(K0 + j * PITCH, 2 * P), :] = _nt(
                _unpacked(fwd_w[...]), ssmk[slot, :, pl.ds(j * P, P)])
            if j % 4 == 3:
                yield

    def shift_conv(c, step):
        for r in range(0, S, step):
            w = [jnp.tile(par[c, j], (step // 8, 1)) for j in range(KS)]
            words = pl.ds(r // 2, step // 2)
            k = _unpacked(ak_w[c % 2, words, :]).astype(F32)
            work[pl.ds(X0 + 8 + r, step), :] = k
            acc = work[pl.ds(X0 + 8 + r - (KS - 1), step), :] * w[KS - 1]
            for j in range(KS - 2, 0, -1):
                acc = acc + work[pl.ds(X0 + 8 + r - j, step), :] * w[j]
            acc = acc + k * w[0]
            v = _unpacked(av_w[c % 2, words, :]).astype(F32)
            kvb[pl.ds(r, step), :] = (acc * v).astype(BF16)
            yield 1

    def chunk_conv():
        for f in range(0, P, 8):
            def re(b, i):
                return pl.ds(b + i * PITCH + f, 8)

            def im(b, i):
                return pl.ds(b + i * PITCH + P + f, 8)

            kc = [work[re(K0, 0), :]] + [
                work[re(K0, j), :] - work[im(K0, j - 1), :] for j in range(1, Q)]
            us = [work[re(U0, i), :] + work[im(U0, i), :] for i in range(Q)]
            yield 2 * Q
            s1 = []
            for a in range(Q):
                t = kc[0] * us[a]
                for j in range(1, a + 1):
                    t = t + kc[j] * us[a - j]
                s1.append(t)
                yield 2 * (a + 1)
            kd = [work[im(K0, 0), :]] + [
                work[im(K0, j), :] + work[re(K0, j - 1), :] for j in range(1, Q)]
            km = [d_ - c_ for c_, d_ in zip(kc, kd)]
            kp = [d_ + c_ for c_, d_ in zip(kc, kd)]
            yield 3 * Q
            ua = [work[re(U0, i), :] for i in range(Q)]
            for a in range(Q):
                t = s1[a]
                for j in range(a + 1):
                    t = t + km[j] * ua[a - j]
                work[im(Z0, a), :] = t
                yield 2 * (a + 1)
            ub = [work[im(U0, i), :] for i in range(Q)]
            for a in range(Q):
                t = s1[a]
                for j in range(a + 1):
                    t = t - kp[j] * ub[a - j]
                work[re(Z0, a), :] = t
                yield 2 * (a + 1)

    xa_copy = pltpu.make_async_copy(x_hbm.at[:, RG - 1], xa_raw, sem_xa)
    small = [
        pltpu.make_async_copy(src, dst, sem_s.at[i]) for i, (src, dst) in enumerate(zip(
            (shift_hbm, ssmd_hbm, mem0_hbm, fwd_hbm, inv_hbm),
            (shift_ref, ssmd_ref, mem0_ref, fwd_ref, inv_ref)))
    ]
    small[0].start()
    small[1].start()
    first_copy(0).start()
    xa_copy.start()
    small[0].wait()
    small[1].wait()
    for g in range(1, NB):
        first_copy(g).start()
    work[pl.ds(X0, 8), :] = jnp.zeros((8, LANES), F32)
    shift = shift_ref[...].astype(F32)
    skip_all = ssmd_ref[...].astype(F32)
    for c in range(NB):
        for j in range(KS):
            par[c, j] = jnp.broadcast_to(shift[j:j + 1, c * LANES:(c + 1) * LANES], (8, LANES))
        par[c, KS] = jnp.broadcast_to(skip_all[c:c + 1, :], (8, LANES))
    xa_copy.wait()
    for cp in small[2:] + stage_copies(0):
        cp.start()
    xa[...] = pltpu.bitcast(xa_raw[...].astype(F32).reshape(NA, D).astype(BF16), U32)

    def warm_up(g, _):
        first_copy(g).wait()
        for _ in project_ahead([(raw0.at[g], 0, g)], 128):
            pass
        return 0

    lax.fori_loop(0, NB, warm_up, 0)
    for cp in small[2:]:
        cp.wait()

    def stage(c, _):
        for cp in stage_copies(c):
            cp.wait()
        slot = c % 2
        pairs = stage_pairs(c)
        ahead = project_ahead(
            [(raw.at[slot, n], m, g) for n, (m, g) in enumerate(pairs)], 64)
        next(ahead)
        per_pair = 2 * NA // 64

        _interleave(_chain(kernel_spectra(slot), _take(ahead, per_pair)), per_pair,
                    shift_conv(c, 32), S // 32)
        for i in range(Q):
            work[ordered(U0 + i * PITCH, 2 * P), :] = _nn(
                _unpacked(fwd_w[...]), _unpacked(kvb_w[pl.ds(i * P // 2, P // 2), :]))
        _interleave(_take(ahead, (len(pairs) - 1) * per_pair - 2), 1.75 * per_pair,
                    chunk_conv(), P // 8 * (5 * Q + 3 * Q * (Q + 1)))
        skip = jnp.tile(par[c, KS], (P // 8, 1))
        for a in range(Q):
            words = pl.ds(a * P // 2, P // 2)
            z = work[pl.ds(Z0 + a * PITCH, 2 * P), :].astype(BF16)
            y = _nn(inv_ref[...], z) + _unpacked(kvb_w[words, :]).astype(F32) * skip
            q = _unpacked(aq_w[slot, words, :]).astype(F32)
            aout[c, pl.ds(a * P, P), :] = (q * y).astype(BF16)

        @pl.when(c + 2 < NB)
        def _():
            for cp in stage_copies(c + 2):
                cp.start()

        @pl.when(c + 2 == NB)
        def _():
            x_copy(0).start()

        @pl.when(c + 1 < NB)
        def _():
            wo_copy(c + 1).start()

        for _ in ahead:
            pass
        return 0

    for cp in stage_copies(1) + [wo_copy(0)]:
        cp.start()
    lax.fori_loop(0, NB, stage, 0)
    for c in range(NB):
        wo_copy(c).wait()
    for g in range(1, XG):
        x_copy(g).start()
    for c in range(NB):
        aout_copy(c).start()

    scale = LANES ** -0.5
    row = lax.broadcasted_iota(jnp.int32, (L, L), 0)
    col = lax.broadcasted_iota(jnp.int32, (L, L), 1)
    mask = (row < M) | (row >= col)

    def segment(s, mem):
        rows = pl.ds(pl.multiple_of(s * seg, seg), seg)
        h = jnp.concatenate(
            [mem, xs[s].astype(F32).reshape(seg - AHEAD, D)], axis=0).astype(BF16)

        def finish(i, late):
            early = work[pl.ds(pl.multiple_of(i * NA + s * AHEAD, AHEAD), AHEAD), :]
            return jnp.concatenate([late, early], axis=0)

        D1, D2 = 2, 4
        HS = H - 8
        proj, prob, acc, heads = {}, {}, {}, []
        for t in range(H + D2):
            if t < H:
                ids = [m * H + t for m in range(3)]
                if t == 0:
                    lo = [_nn(h[:, :D // 2], _unpacked(wqkv_w[i, :D // 4, :])) for i in ids]
                    late = [_nn(h[:, D // 2:], _unpacked(wqkv_w[i, D // 4:, :])) + part
                            for i, part in zip(ids, lo)]
                else:
                    late = [_nn(h, _unpacked(wqkv_w[i])) for i in ids]
                q, k, v = (finish(i, y) for i, y in zip(ids, late))
                proj[t] = (q, k.astype(BF16), v.astype(BF16))
            else:
                for j in range((t - H) * NB // D2, (t - H + 1) * NB // D2):
                    acc[j] = _nn(jnp.concatenate(heads[:HS], axis=1),
                                 _unpacked(wo_w[j, :HS * LANES // 2, :]))
            if 0 <= t - D1 < H:
                q, k, v = proj.pop(t - D1)
                sc = jnp.where(mask, _nt(q, k) * scale, -1e9)
                e = jnp.exp(sc - jnp.max(sc, axis=-1, keepdims=True))
                den = jnp.sum(e, axis=-1, keepdims=True)
                prob[t - D1] = (e * pltpu.reciprocal(den, approx=False, full_range=False), v)
            for u in [u for u in prob if u <= (t - D2 if t < H + D2 - 2 else H)]:
                p, v = prob.pop(u)
                heads.append(_nn(p, v))

        new_mem = []
        for j in range(NB):
            res = _nn(jnp.concatenate(heads[HS:], axis=1),
                      _unpacked(wo_w[j, HS * LANES // 2:, :])) + acc[j]
            new_mem.append(res[:M])
            bout[rows, pl.ds(j * LANES, LANES)] = res[M:].astype(BF16)
        bout_copy(rows).start()
        return jnp.concatenate(new_mem, axis=1)

    def segments(i, mem):
        @pl.when(i % (SPG // UNROLL) == 0)
        def _():
            x_copy(i // (SPG // UNROLL)).wait()

        for u in range(UNROLL):
            mem = segment(i * UNROLL + u, mem)
        return mem

    lax.fori_loop(0, n_seg // UNROLL, segments, mem0_ref[...].astype(F32))
    for c in range(NB):
        aout_copy(c).wait()
    bout_copy(pl.ds(0, S)).wait()


@functools.partial(jax.jit, static_argnames=("B_seg_len",))
def pallas_concat_heads__ssm_conv_h3__memory_aug_recurrent_mem_tr__prompt_kernel(
    A_q, A_k, A_v, A_shift_k, A_ssm_k, A_ssm_D,
    B_x, B_mem0, B_Wq, B_Wk, B_Wv, B_Wo, B_seg_len,
):
    B, S, D = A_q.shape
    _, H, Dh = B_Wq.shape
    M = B_mem0.shape[1]
    KS = A_shift_k.shape[1]
    seg = int(B_seg_len)
    assert B == 1 and Dh == LANES and B_x.shape == (B, S, D)
    NB = D // LANES
    n_seg = S // seg
    NA = n_seg * AHEAD
    n_pairs = 3 * (H // 2 // NB) - 1
    fwd, inv = _dft_matrices()

    hbm = pl.BlockSpec(memory_space=pl.ANY)
    out = pl.pallas_call(
        functools.partial(_kernel, S=S, D=D, H=H, M=M, seg=seg),
        out_shape=jax.ShapeDtypeStruct((S, 2 * D), BF16),
        in_specs=[hbm] * 14 + [pl.BlockSpec(memory_space=pltpu.SMEM)],
        out_specs=hbm,
        scratch_shapes=[
            pltpu.VMEM((KS, D), BF16),
            pltpu.VMEM((NB, LANES), BF16),
            pltpu.VMEM((M, D), BF16),
            pltpu.VMEM(fwd.shape, BF16),
            pltpu.VMEM(inv.shape, BF16),
            pltpu.VMEM((2, S, LANES), BF16),
            pltpu.VMEM((2, S, LANES), BF16),
            pltpu.VMEM((2, S, LANES), BF16),
            pltpu.VMEM((2, LANES, S), BF16),
            pltpu.VMEM((NB, S, LANES), BF16),
            pltpu.VMEM((NB, KS + 1, 8, LANES), F32),
            pltpu.VMEM((S, LANES), BF16),
            pltpu.VMEM((3 * H * NA + 3 * (S // P) * PITCH + 8 + S, LANES), F32),
            pltpu.VMEM((NB, D, LANES), U32),
            pltpu.VMEM((2, n_pairs, D, LANES), U32),
            pltpu.VMEM((3 * H, D, LANES), BF16),
            pltpu.VMEM((NB, H * Dh, LANES), BF16),
            pltpu.VMEM((n_seg, AHEAD, D), BF16),
            pltpu.VMEM((NA // 2, D), U32),
            pltpu.VMEM((n_seg, seg // AHEAD - 1, AHEAD, D), BF16),
            pltpu.VMEM((S, D), BF16),
            pltpu.SemaphoreType.DMA((5,)),
            pltpu.SemaphoreType.DMA((2, 4)),
            pltpu.SemaphoreType.DMA((NB,)),
            pltpu.SemaphoreType.DMA((2, n_pairs)),
            pltpu.SemaphoreType.DMA((NB,)),
            pltpu.SemaphoreType.DMA(()),
            pltpu.SemaphoreType.DMA((XG,)),
            pltpu.SemaphoreType.DMA((NB,)),
            pltpu.SemaphoreType.DMA(()),
        ],
        compiler_params=pltpu.CompilerParams(
            vmem_limit_bytes=112 * 1024 * 1024, disable_bounds_checks=True),
        name="h3_rmt_concat",
    )(
        A_q.reshape(S, D), A_k.reshape(S, D), A_v.reshape(S, D),
        A_shift_k.T, A_ssm_k, A_ssm_D.reshape(NB, LANES),
        B_x.reshape(n_seg, seg // AHEAD, AHEAD, D), B_mem0.reshape(M, D),
        B_Wq, B_Wk, B_Wv, B_Wo.reshape(H * Dh, D),
        fwd, inv, np.zeros((1,), np.int32),
    )
    return out.reshape(B, S, 2 * D)
```
